```python
import os as _os
_os.environ.setdefault("JAX_PLATFORMS", "cpu")
import jax
import jax.numpy as jnp

def _softmax(x, axis=-1):
    return jax.nn.softmax(x, axis=axis)
def _gelu(x):
    return jax.nn.gelu(x, approximate=True)
def _silu(x):
    return jax.nn.silu(x)
def _sigmoid(x):
    return jax.nn.sigmoid(x)
def _layernorm(x, axis=-1, eps=1e-5):
    m = jnp.mean(x, axis=axis, keepdims=True)
    v = jnp.var(x, axis=axis, keepdims=True)
    return (x - m) / jnp.sqrt(v + eps)
def _scatter_add(tgt, idx, src, axis=0):
    return tgt.at[idx].add(src)
def _segment_sum(src, seg, n):
    return jax.ops.segment_sum(src, seg, n)
class _Rng:
    def __init__(self, key):
        self._k = key
    def _next(self):
        self._k, sub = jax.random.split(self._k)
        return sub
    def normal(self, shape):
        return jax.random.normal(self._next(), shape, dtype=jnp.bfloat16)
    def randint(self, lo, hi, shape):
        return jax.random.randint(self._next(), shape, lo, hi, dtype=jnp.int32)
    def uniform(self, shape, lo=0.0, hi=1.0):
        return jax.random.uniform(self._next(), shape, jnp.bfloat16, lo, hi)
    def permutation(self, n):
        return jax.random.permutation(self._next(), n)


kernel_name = 'sequential_preLN__linear_kernel_hedgehog__geglu_ffn__prompt'

def setup_inputs():
    _rng = _Rng(jax.random.key(int.from_bytes(__import__("os").urandom(4), "little")))
    _w = (lambda a: (lambda t: t.astype(jnp.bfloat16) if jnp.issubdtype(t.dtype, jnp.floating) else t)(jnp.asarray(a)))
    def _A_setup():
        B, S, D, H = 1, 2048, 640, 32
        Dh = D // H
        return {
            "x": _w((lambda *s: _rng.normal(s) * 0.05)(B, S, D)),
            "wqkv": _w((lambda *s: _rng.normal(s) * 0.2)(D, 3 * D)),
            "w_phi": _w((lambda *s: _rng.normal(s) * 0.2)(H, Dh, Dh) * (Dh ** -0.5)),
            "wo": _w((lambda *s: _rng.normal(s) * 0.05)(D, D)),
        }
    _A_in = _A_setup()

    def _B_setup():
        B, S, D, F = 1, 2048, 640, 1536
        return {
            "x": _w((lambda *s: _rng.normal(s) * 0.05)(B, S, D)),
            "w_gate": _w((lambda *s: _rng.normal(s) * 0.05)(D, F)),
            "w_up": _w((lambda *s: _rng.normal(s) * 0.05)(D, F)),
            "w_down": _w((lambda *s: _rng.normal(s) * 0.05)(F, D)),
        }
    _B_in = _B_setup()

    return {
        "A_x": _A_in["x"],
        "A_wqkv": _A_in["wqkv"],
        "A_w_phi": _A_in["w_phi"],
        "A_wo": _A_in["wo"],
        "B_x": _B_in["x"],
        "B_w_gate": _B_in["w_gate"],
        "B_w_up": _B_in["w_up"],
        "B_w_down": _B_in["w_down"],
    }

def reference(A_x, A_wqkv, A_w_phi, A_wo, B_x, B_w_gate, B_w_up, B_w_down):
    def _A_ref(x, wqkv, w_phi, wo):
        B, S, D = x.shape
        H = 32; Dh = D // H
        qkv = (lambda x, *d: x.transpose(*d))((x @ wqkv).reshape(B, S, 3, H, Dh), 2, 0, 3, 1, 4)
        q, k, v = qkv[0], qkv[1], qkv[2]
        pq = jnp.einsum("bhsd,hdf->bhsf", q, w_phi)
        pk = jnp.einsum("bhsd,hdf->bhsf", k, w_phi)
        phi_q = jnp.concatenate([_softmax(pq, axis=-1), _softmax(-pq, axis=-1)], axis=-1)
        phi_k = jnp.concatenate([_softmax(pk, axis=-1), _softmax(-pk, axis=-1)], axis=-1)
        kv = jnp.einsum("bhsf,bhsd->bhfd", phi_k, v)
        z  = jnp.einsum("bhsf->bhf", phi_k)
        num = jnp.einsum("bhqf,bhfd->bhqd", phi_q, kv)
        den = jnp.einsum("bhqf,bhf->bhq", phi_q, z)[..., None] + 1e-6
        o = num / den
        return (lambda x, *d: x.transpose(*d))(o, 0, 2, 1, 3).reshape(B, S, D) @ wo

    def _B_ref(x, w_gate, w_up, w_down):
        return (_gelu(x @ w_gate) * (x @ w_up)) @ w_down

    x = A_x
    h = x + _A_ref(_layernorm(x, axis=-1), A_wqkv, A_w_phi, A_wo)
    h2 = h + _B_ref(_layernorm(h, axis=-1), B_w_gate, B_w_up, B_w_down)
    return h2
```

```python
import functools
import jax
import jax.numpy as jnp
from jax import lax
import jax.experimental.pallas as pl
import jax.experimental.pallas.tpu as pltpu

S, D, H, DH, F = 2048, 640, 32, 20, 1536
NG = H // 2
EPS = 1e-5
NT = (((1,), (1,)), ((), ()))
f32, bf16 = jnp.float32, jnp.bfloat16

def _ranges(rows_per_group_in_tile_space, rows_per_group_out, ntiles):
    out = []
    for i in range(ntiles):
        g0 = (128 * i) // rows_per_group_in_tile_space
        g1 = (128 * i + 127) // rows_per_group_in_tile_space
        r0 = (g0 * rows_per_group_out) // 16 * 16
        r1 = -((-(g1 + 1) * rows_per_group_out) // 16) * 16
        out.append((r0, r1))
    return out

KV_R = _ranges(80, 40, 10)
FOLD_R = _ranges(40, 40, 5)


def _assemble(parts, ranges, total):
    cuts = sorted({0, total} | {r for rr in ranges for r in rr})
    segs = []
    for a, b in zip(cuts[:-1], cuts[1:]):
        acc = None
        for p, (r0, r1) in zip(parts, ranges):
            if r0 <= a and b <= r1:
                piece = p[a - r0:b - r0]
                acc = piece if acc is None else acc + piece
        segs.append(acc)
    return jnp.concatenate(segs, axis=0)


def _layernorm(x):
    m = jnp.mean(x, axis=-1, keepdims=True)
    xc = x - m
    v = jnp.mean(xc * xc, axis=-1, keepdims=True)
    return xc * lax.rsqrt(v + EPS)


def _allred(x, op):
    x = op(x, pltpu.roll(x, 4, 1))
    return op(x, pltpu.roll(x, 2, 1))


def _exps(pT):
    ts = pT.shape[1]
    p = pT.reshape(NG, 5, 8, ts)
    mx = _allred(jnp.max(p, axis=1), jnp.maximum)
    mn = _allred(jnp.min(p, axis=1), jnp.minimum)
    ep = jnp.exp(p - mx[:, None])
    en = jnp.exp(mn[:, None] - p)
    sp = _allred(jnp.sum(ep, axis=1), jnp.add)
    sn = _allred(jnp.sum(en, axis=1), jnp.add)
    return ep, en, sp, sn


def _gelu(x):
    c = 0.7978845608028654
    return 0.5 * x * (1.0 + jnp.tanh(c * (x + 0.044715 * (x * x * x))))


def make_kernel(TS1, TS2):
    n1, n2 = S // TS1, S // TS2
    NX = 4
    XC = S // NX

    def kernel(x_hbm, wqkv_hbm, wphi_hbm, wo_hbm, wg_hbm, wu_hbm, wd_hbm, o_hbm,
               x_v, wqkv_v, wphi_v, wo_v, wg_v, wu_v, wd_v, out_v,
               a_s, wkvT, wqT, xn_s, kv_acc, kvT, z_acc, sems, osems):
        cp_phi = pltpu.make_async_copy(wphi_hbm, wphi_v, sems.at[0])
        cp_k = pltpu.make_async_copy(wqkv_hbm.at[:, pl.ds(D, D)], wqkv_v.at[:, pl.ds(D, D)], sems.at[1])
        cp_v = pltpu.make_async_copy(wqkv_hbm.at[:, pl.ds(2 * D, D)], wqkv_v.at[:, pl.ds(2 * D, D)], sems.at[2])
        cp_q = pltpu.make_async_copy(wqkv_hbm.at[:, pl.ds(0, D)], wqkv_v.at[:, pl.ds(0, D)], sems.at[3])
        cp_wo = pltpu.make_async_copy(wo_hbm, wo_v, sems.at[4])
        cp_wg = pltpu.make_async_copy(wg_hbm, wg_v, sems.at[5])
        cp_wu = pltpu.make_async_copy(wu_hbm, wu_v, sems.at[6])
        cp_wd = pltpu.make_async_copy(wd_hbm, wd_v, sems.at[7])
        cp_x = [pltpu.make_async_copy(x_hbm.at[0, pl.ds(c * XC, XC)], x_v.at[pl.ds(c * XC, XC)], sems.at[8 + c])
                for c in range(NX)]
        cp_phi.start(); cp_k.start(); cp_v.start()
        for c in cp_x:
            c.start()
        cp_q.start()

        cp_phi.wait()
        for h in range(H):
            a_s[pl.ds(DH * h, DH), :] = wphi_v[h].astype(f32)
        a = a_s[...].astype(bf16)
        r = lax.broadcasted_iota(jnp.int32, (48, DH), 0)
        k = lax.broadcasted_iota(jnp.int32, (48, DH), 1)
        onehot = jnp.where(k == r // 2, 1.0, 0.0).astype(bf16)
        trep = lax.dot_general(onehot, a, NT, preferred_element_type=f32)[:40]
        bdts = []
        for t, (r0, r1) in enumerate(FOLD_R):
            g0 = r0 // 40
            g1 = -(-r1 // 40)
            blk = jnp.concatenate([trep[:, 128 * t:128 * t + 128]] * (g1 - g0), axis=0)
            blk = blk[r0 - 40 * g0:r1 - 40 * g0]
            rr = lax.broadcasted_iota(jnp.int32, blk.shape, 0) + r0
            cc = lax.broadcasted_iota(jnp.int32, blk.shape, 1) + 128 * t
            keep = (2 * (rr // 40) + rr % 2) == cc // DH
            bdts.append(jnp.where(keep, blk, 0.0).astype(bf16))

        def fold(off):
            parts = [lax.dot_general(bdts[t], wqkv_v[:, off + 128 * t:off + 128 * t + 128], NT,
                                     preferred_element_type=f32) for t in range(5)]
            return _assemble(parts, FOLD_R, D).astype(bf16)

        cp_k.wait()
        wkvT[0:D, :] = fold(D)
        cp_v.wait()
        wkvT[D:2 * D, :] = wqkv_v[:, 2 * D:3 * D].T
        cp_wo.start(); cp_wg.start(); cp_wu.start(); cp_wd.start()
        cp_q.wait()
        wqT[...] = fold(0)
        kv_acc[...] = jnp.zeros_like(kv_acc)
        z_acc[...] = jnp.zeros_like(z_acc)
        for c in cp_x:
            c.wait()

        offs = [0]
        for (r0, r1) in KV_R:
            offs.append(offs[-1] + r1 - r0)

        def p1(t, carry):
            row = pl.multiple_of(t * TS1, TS1)
            xn = _layernorm(x_v[pl.ds(row, TS1), :].astype(f32)).astype(bf16)
            xn_s[pl.ds(row, TS1), :] = xn
            kv = lax.dot_general(wkvT[...], xn, NT, preferred_element_type=f32)
            ep, en, sp, sn = _exps(kv[:D])
            phi = jnp.concatenate([ep * (1.0 / sp)[:, None], en * (1.0 / sn)[:, None]], axis=1)
            phi = phi.reshape(2 * D, TS1)
            zs = phi[:, 0:128]
            for j in range(1, TS1 // 128):
                zs = zs + phi[:, 128 * j:128 * j + 128]
            z_acc[...] += zs
            phib = phi.astype(bf16)
            vT = kv[D:].astype(bf16)
            for i, (r0, r1) in enumerate(KV_R):
                kv_acc[offs[i]:offs[i + 1], :] += lax.dot_general(
                    vT[r0:r1], phib[128 * i:128 * i + 128], NT, preferred_element_type=f32)
            return carry
        lax.fori_loop(0, n1, p1, 0)

        for i, (r0, r1) in enumerate(KV_R):
            blk = kv_acc[offs[i]:offs[i + 1], :]
            rr = lax.broadcasted_iota(jnp.int32, blk.shape, 0) + r0
            cc = lax.broadcasted_iota(jnp.int32, blk.shape, 1) + 128 * i
            keep = (rr // DH) == 2 * (cc // 80) + cc % 2
            kvT[offs[i]:offs[i + 1], :] = jnp.where(keep, blk, 0.0).astype(bf16)
        z_acc[...] = jnp.broadcast_to(jnp.sum(z_acc[...], axis=1, keepdims=True), z_acc.shape)

        cp_wo.wait(); cp_wg.wait(); cp_wu.wait(); cp_wd.wait()

        def out_copy(t):
            row = pl.multiple_of(t * TS2, TS2)
            return pltpu.make_async_copy(out_v.at[pl.ds(row, TS2)], o_hbm.at[0, pl.ds(row, TS2)], osems.at[t])

        def p2(t, carry):
            row = pl.multiple_of(t * TS2, TS2)
            xn = xn_s[pl.ds(row, TS2), :]
            pq = lax.dot_general(wqT[...], xn, NT, preferred_element_type=f32)
            ep, en, sp, sn = _exps(pq)
            z = z_acc[...].reshape(NG, 10, 8, 128)
            z = jnp.concatenate([z] * (TS2 // 128), axis=-1)
            rp, rn = 1.0 / sp, 1.0 / sn
            dp = jnp.sum(ep * z[:, :5], axis=1)
            dn = jnp.sum(en * z[:, 5:], axis=1)
            den = _allred(dp * rp + dn * rn, jnp.add) + 1e-6
            rd = 1.0 / den
            phi = jnp.concatenate([ep * (rp * rd)[:, None], en * (rn * rd)[:, None]], axis=1)
            phib = phi.reshape(2 * D, TS2).astype(bf16)
            parts = [jnp.dot(kvT[offs[i]:offs[i + 1], :], phib[128 * i:128 * i + 128],
                             preferred_element_type=f32) for i in range(10)]
            oT = _assemble(parts, KV_R, D)
            o = oT.T.astype(bf16)
            h = x_v[pl.ds(row, TS2), :].astype(f32) + jnp.dot(o, wo_v[...], preferred_element_type=f32)
            hn = _layernorm(h).astype(bf16)
            g = jnp.dot(hn, wg_v[...], preferred_element_type=f32)
            u = jnp.dot(hn, wu_v[...], preferred_element_type=f32)
            act = (_gelu(g) * u).astype(bf16)
            y = h + jnp.dot(act, wd_v[...], preferred_element_type=f32)
            out_v[pl.ds(row, TS2), :] = y.astype(bf16)
            out_copy(t).start()
            return carry
        lax.fori_loop(0, n2, p2, 0)
        for t in range(n2):
            out_copy(t).wait()

    kv_rows = sum(r1 - r0 for r0, r1 in KV_R)
    scratch = [
        pltpu.VMEM((S, D), bf16),
        pltpu.VMEM((D, 3 * D), bf16),
        pltpu.VMEM((H, DH, DH), bf16),
        pltpu.VMEM((D, D), bf16),
        pltpu.VMEM((D, F), bf16),
        pltpu.VMEM((D, F), bf16),
        pltpu.VMEM((F, D), bf16),
        pltpu.VMEM((S, D), bf16),
        pltpu.VMEM((D, DH), f32),
        pltpu.VMEM((2 * D, D), bf16),
        pltpu.VMEM((D, D), bf16),
        pltpu.VMEM((S, D), bf16),
        pltpu.VMEM((kv_rows, 128), f32),
        pltpu.VMEM((kv_rows, 128), bf16),
        pltpu.VMEM((2 * D, 128), f32),
        pltpu.SemaphoreType.DMA((8 + NX,)),
        pltpu.SemaphoreType.DMA((n2,)),
    ]
    return kernel, scratch


def build(TS1=256, TS2=256):
    @jax.jit
    def fn(A_x, A_wqkv, A_w_phi, A_wo, B_x, B_w_gate, B_w_up, B_w_down):
        kernel, scratch = make_kernel(TS1, TS2)
        return pl.pallas_call(
            kernel,
            out_shape=jax.ShapeDtypeStruct(A_x.shape, A_x.dtype),
            in_specs=[pl.BlockSpec(memory_space=pl.ANY)] * 7,
            out_specs=pl.BlockSpec(memory_space=pl.ANY),
            scratch_shapes=scratch,
            compiler_params=pltpu.CompilerParams(vmem_limit_bytes=100 * 1024 * 1024),
        )(A_x, A_wqkv, A_w_phi, A_wo, B_w_gate, B_w_up, B_w_down)
    return fn


_impl = build(TS1=512,TS2=512)


@jax.jit
def pallas_sequential_preLN__linear_kernel_hedgehog__geglu_ffn__prompt_kernel(
    A_x: jax.Array,
    A_wqkv: jax.Array,
    A_w_phi: jax.Array,
    A_wo: jax.Array,
    B_x: jax.Array,
    B_w_gate: jax.Array,
    B_w_up: jax.Array,
    B_w_down: jax.Array,
):
    return _impl(A_x, A_wqkv, A_w_phi, A_wo, B_x, B_w_gate, B_w_up, B_w_down)
```

```python
import jax
import jax.numpy as jnp
from jax import lax
import jax.experimental.pallas as pl
import jax.experimental.pallas.tpu as pltpu

S, D, H, DH, F = 2048, 640, 32, 20, 1536
NG = H // 2
EPS = 1e-5
LOG2E = 1.4426950408889634
NT = (((1,), (1,)), ((), ()))
f32, bf16 = jnp.float32, jnp.bfloat16

TS = 512
NTILE = S // TS
HX = TS // 2
VA = 256
A1, B1 = 512, 448
NA = 4
OCOLS = (0, 256, 512, 640)
NOC = len(OCOLS) - 1


def _ranges(rows_in, rows_out, ntiles, align):
    out = []
    for i in range(ntiles):
        g0 = (128 * i) // rows_in
        g1 = (128 * i + 127) // rows_in
        r0 = (g0 * rows_out) // align * align
        r1 = -((-(g1 + 1) * rows_out) // align) * align
        out.append((r0, r1))
    return out


KV_R = _ranges(80, 40, 10, 8)
KV_L = [-(-(r1 - r0 + 8) // 16) * 16 for r0, r1 in KV_R]
KV_OFF = [sum(KV_L[:i]) for i in range(11)]
FOLD_R = _ranges(40, 40, 5, 16)
FOLD_OFF = [sum(r1 - r0 for r0, r1 in FOLD_R[:i]) for i in range(6)]


def _assemble(parts, ranges, total):
    cuts = sorted({0, total} | {r for rr in ranges for r in rr})
    segs = []
    for a, b in zip(cuts[:-1], cuts[1:]):
        acc = None
        for p, (r0, r1) in zip(parts, ranges):
            if r0 <= a and b <= r1:
                piece = p[a - r0:b - r0]
                acc = piece if acc is None else acc + piece
        segs.append(acc)
    return jnp.concatenate(segs, axis=0)


def _layernorm(x):
    m = jnp.sum(x, axis=-1, keepdims=True) * (1.0 / D)
    xc = x - m
    v = jnp.sum(xc * xc, axis=-1, keepdims=True) * (1.0 / D)
    return xc * lax.rsqrt(v + EPS)


def _allred(x, op):
    x = op(x, pltpu.roll(x, 4, 1))
    return op(x, pltpu.roll(x, 2, 1))


def _feat(pT):
    ts = pT.shape[1]
    p = pT.reshape(NG, 5, 8, ts)
    mx = _allred(jnp.max(p, axis=1), jnp.maximum)
    mn = _allred(jnp.min(p, axis=1), jnp.minimum)
    ep = jnp.exp2(p - mx[:, None])
    en = jnp.exp2(mn[:, None] - p)
    sp = _allred(jnp.sum(ep, axis=1), jnp.add)
    sn = _allred(jnp.sum(en, axis=1), jnp.add)
    rp, rn = pl.reciprocal(sp, approx=True), pl.reciprocal(sn, approx=True)
    phi = jnp.concatenate([ep * rp[:, None], en * rn[:, None]], axis=1).reshape(2 * D, ts)
    return [phi[128 * i:128 * i + 128] for i in range(10)]


def _gelu(x):
    c = 0.7978845608028654
    return 0.5 * x * (1.0 + jnp.tanh(c * (x + 0.044715 * (x * x * x))))


def _iota(shape, dim):
    return lax.broadcasted_iota(jnp.int32, shape, dim)


def _dot(a, b):
    return jnp.dot(a, b, preferred_element_type=f32)


def _dot_nt(a, b):
    return lax.dot_general(a, b, NT, preferred_element_type=f32)


def _kernel(x_hbm, wqkv_hbm, wphi_hbm, wo_hbm, wg_hbm, wu_hbm, wd_hbm, o_hbm,
            x_v, wqkv_v, wphi_v, wo_v, wg_v, wu_v, wd_v, out_v,
            wkT, wvT, wqT, xn_s, kvT, kv_acc, bdt_s, lhs_s, fq_s, sems, osems):
    n = NTILE

    @pl.when(pl.program_id(0) == 0)
    def _phase1():
        def wblock(r0, nr, c0, s):
            return pltpu.make_async_copy(wqkv_hbm.at[pl.ds(r0, nr), pl.ds(c0, D)],
                                         wqkv_v.at[pl.ds(r0, nr), pl.ds(c0, D)], sems.at[s])

        def xrows(row, nr, s):
            return pltpu.make_async_copy(x_hbm.at[0, pl.ds(row, nr)], x_v.at[pl.ds(row, nr)], sems.at[s])

        def cp_x(t):
            return xrows(pl.multiple_of(t * TS, TS), TS, 10 + t)

        cp_phi = pltpu.make_async_copy(wphi_hbm, wphi_v, sems.at[0])
        cp_x0a, cp_x0b = xrows(0, HX, 9), xrows(HX, HX, 10)
        cp_va, cp_vb = wblock(0, VA, 2 * D, 1), wblock(VA, D - VA, 2 * D, 2)
        cp_k, cp_q = wblock(0, D, D, 3), wblock(0, D, 0, 4)
        cp_ffn = [pltpu.make_async_copy(src, dst, sems.at[5 + j]) for j, (src, dst) in enumerate(
            [(wo_hbm, wo_v), (wg_hbm, wg_v), (wu_hbm, wu_v), (wd_hbm, wd_v)])]
        for c in [cp_phi, cp_x0a, cp_x0b, cp_va, cp_vb, cp_k, cp_q] + [cp_x(t) for t in range(1, n)] + cp_ffn:
            c.start()

        def put_lhs(t, vT):
            for i, (r0, r1) in enumerate(KV_R):
                lhs_s[t % 2, KV_OFF[i]:KV_OFF[i + 1], :] = jnp.concatenate(
                    [vT[r0:r1], jnp.ones((KV_L[i] - (r1 - r0), TS), f32)], axis=0).astype(bf16)

        def put_feat(slot, phi):
            for i in range(10):
                fq_s[slot, 128 * i:128 * i + 128, :] = phi[i].astype(bf16)

        def put_kv(kv):
            for i in range(10):
                kv_acc[KV_OFF[i]:KV_OFF[i + 1], :] = kv[i]

        def PK(t):
            return _feat(_dot_nt(wkT[...], xn_s[t % 2]))

        def PQ(t):
            put_feat(t, _feat(_dot_nt(wqT[...], xn_s[t % 2])))

        def LNPV(t):
            row = pl.multiple_of(t * TS, TS)
            xn = _layernorm(x_v[pl.ds(row, TS), :].astype(f32)).astype(bf16)
            xn_s[t % 2] = xn
            put_lhs(t, _dot_nt(wvT[...], xn))

        def KV(t, phi):
            return [kv_acc[KV_OFF[i]:KV_OFF[i + 1], :]
                    + _dot_nt(lhs_s[t % 2, KV_OFF[i]:KV_OFF[i + 1], :], phi[i].astype(bf16))
                    for i in range(10)]

        def fold(off):
            parts = [_dot_nt(bdt_s[FOLD_OFF[t]:FOLD_OFF[t + 1], :],
                             wqkv_v[:, off + 128 * t:off + 128 * t + 128]) for t in range(5)]
            return (_assemble(parts, FOLD_R, D) * LOG2E).astype(bf16)

        kk = _iota((D, 1), 0)
        wqT[...] = jnp.where(_iota((1, D), 1) == DH * (kk % H) + kk // H, 1.0, 0.0).astype(bf16)
        onehot = jnp.where(_iota((48, DH), 1) == _iota((48, DH), 0) // 2, 1.0, 0.0).astype(bf16)
        cp_phi.wait()
        q = jnp.concatenate([wphi_v[d].astype(f32) for d in range(DH)], axis=1).astype(bf16)
        trep = _dot(_dot(onehot, q).astype(bf16), wqT[...])[:40]
        hc = _iota((1, D), 1) // DH
        trep = jnp.where(_iota((40, 1), 0) % 2 == hc % 2, trep, 0.0)
        for t, (r0, r1) in enumerate(FOLD_R):
            g0, g1 = r0 // 40, -(-r1 // 40)
            tt, gc = trep[:, 128 * t:128 * t + 128], hc[:, 128 * t:128 * t + 128] // 2
            blk = jnp.concatenate([jnp.where(gc == g, tt, 0.0) for g in range(g0, g1)], axis=0)
            bdt_s[FOLD_OFF[t]:FOLD_OFF[t + 1], :] = blk[r0 - 40 * g0:r1 - 40 * g0].astype(bf16)

        def pva(r0, r1):
            return _dot_nt(wvT[r0:r1, 0:VA], xn_s[0, :, 0:VA])

        def pvb(r0, r1):
            return _dot_nt(wvT[r0:r1, VA:D], xn_s[0, :, VA:D])

        cp_x0a.wait()
        xn_s[0, 0:HX, :] = _layernorm(x_v[0:HX, :].astype(f32)).astype(bf16)
        cp_x0b.wait()
        xn_s[0, HX:TS, :] = _layernorm(x_v[HX:TS, :].astype(f32)).astype(bf16)
        cp_va.wait()
        wvT[:, 0:VA] = wqkv_v[0:VA, 2 * D:3 * D].T
        pa = pva(0, A1)
        cp_vb.wait()
        pa = jnp.concatenate([pa, pva(A1, D)], axis=0)
        wvT[:, VA:D] = wqkv_v[VA:D, 2 * D:3 * D].T
        v0 = pa[0:B1] + pvb(0, B1)
        cp_k.wait()
        wkT[...] = fold(D)
        put_feat(n - 1, PK(0))
        put_lhs(0, jnp.concatenate([v0, pa[B1:D] + pvb(B1, D)], axis=0))
        cp_q.wait()
        cp_x(1).wait()
        wqT[...] = fold(0)
        PQ(0)
        put_kv([_dot_nt(lhs_s[0, KV_OFF[i]:KV_OFF[i + 1], :], fq_s[n - 1, 128 * i:128 * i + 128, :])
                for i in range(10)])
        LNPV(1)

        def p1(t, carry):
            cp_x(t + 1).wait()
            fk = PK(t)
            PQ(t)
            kv = KV(t, fk)
            LNPV(t + 1)
            put_kv(kv)
            return carry
        lax.fori_loop(1, n - 1, p1, 0)

        fk = PK(n - 1)
        PQ(n - 1)
        kv = KV(n - 1, fk)
        for i, (r0, r1) in enumerate(KV_R):
            m = r1 - r0
            cc = _iota((1, 128), 1) + 128 * i
            head_c = 2 * (cc // 80) + cc % 2
            dlt = _iota((m, 1), 0) - (DH * head_c - r0)
            main = jnp.where(jnp.logical_and(dlt >= 0, dlt < DH), kv[i][:m], 0.0)
            hb = 16 * (i // 5) + (8 if i % 5 >= 3 else 0)
            zr = jnp.where(_iota((KV_L[i] - m, 1), 0) + hb == head_c, kv[i][m:], 0.0)
            kvT[KV_OFF[i]:KV_OFF[i + 1], :] = jnp.concatenate([main, zr], axis=0).astype(bf16)
        for c in cp_ffn:
            c.wait()

    @pl.when(pl.program_id(0) == 1)
    def _phase2():
        def out_copy(t, c):
            row = pl.multiple_of(t * TS, TS)
            c0, c1 = OCOLS[c], OCOLS[c + 1]
            return pltpu.make_async_copy(out_v.at[pl.ds(row, TS), pl.ds(c0, c1 - c0)],
                                         o_hbm.at[0, pl.ds(row, TS), pl.ds(c0, c1 - c0)],
                                         osems.at[t * NOC + c])

        def attn_o(t, c0, c1):
            m = c1 - c0
            parts = [_dot(kvT[KV_OFF[i]:KV_OFF[i + 1], :], fq_s[t, 128 * i:128 * i + 128, c0:c1])
                     for i in range(10)]
            num = _assemble(parts, KV_R, D)
            dn = [p[r1 - r0:] for p, (r0, r1) in zip(parts, KV_R)]
            lo = _iota((8, m), 0) < 4
            scale = []
            for b in range(2):
                d = dn[5 * b:5 * b + 5]
                for den in (d[0][:8] + d[1] + d[2][:8], d[2][8:] + d[3] + d[4][:8]):
                    rd = 1.0 / (den + 1e-6)
                    for g in range(4):
                        a0 = jnp.broadcast_to(rd[2 * g:2 * g + 1], (8, m))
                        a1 = jnp.broadcast_to(rd[2 * g + 1:2 * g + 2], (8, m))
                        scale += [a0, a0, jnp.where(lo, a0, a1), a1, a1]
            return (num * jnp.concatenate(scale, axis=0)).T.astype(bf16)

        def p2(t, carry):
            row = pl.multiple_of(t * TS, TS)
            ma = TS // NA
            os_ = [attn_o(t, j * ma, (j + 1) * ma) for j in range(NA)]
            hs = [x_v[pl.ds(row + j * ma, ma), :].astype(f32) + _dot(os_[j], wo_v[...]) for j in range(NA)]
            hn = jnp.concatenate([_layernorm(h) for h in hs], axis=0).astype(bf16)
            h = jnp.concatenate(hs, axis=0)
            g = _dot(hn, wg_v[...])
            u = _dot(hn, wu_v[...])
            act = (_gelu(g) * u).astype(bf16)
            for c in range(NOC):
                c0, c1 = OCOLS[c], OCOLS[c + 1]
                out_v[pl.ds(row, TS), c0:c1] = (h[:, c0:c1] + _dot(act, wd_v[:, c0:c1])).astype(bf16)
                out_copy(t, c).start()
            return carry

        lax.fori_loop(0, n, p2, 0)
        for t in range(n):
            for c in range(NOC):
                out_copy(t, c).wait()


_SCRATCH = [
    pltpu.VMEM((S, D), bf16),
    pltpu.VMEM((D, 3 * D), bf16),
    pltpu.VMEM((DH, DH, H), bf16),
    pltpu.VMEM((D, D), bf16),
    pltpu.VMEM((D, F), bf16),
    pltpu.VMEM((D, F), bf16),
    pltpu.VMEM((F, D), bf16),
    pltpu.VMEM((S, D), bf16),
    pltpu.VMEM((D, D), bf16),
    pltpu.VMEM((D, D), bf16),
    pltpu.VMEM((D, D), bf16),
    pltpu.VMEM((2, TS, D), bf16),
    pltpu.VMEM((KV_OFF[-1], 128), bf16),
    pltpu.VMEM((KV_OFF[-1], 128), f32),
    pltpu.VMEM((FOLD_OFF[-1], 128), bf16),
    pltpu.VMEM((2, KV_OFF[-1], TS), bf16),
    pltpu.VMEM((NTILE, 2 * D, TS), bf16),
    pltpu.SemaphoreType.DMA((10 + NTILE,)),
    pltpu.SemaphoreType.DMA((NTILE * NOC,)),
]


@jax.jit
def pallas_sequential_preLN__linear_kernel_hedgehog__geglu_ffn__prompt_kernel(
    A_x: jax.Array,
    A_wqkv: jax.Array,
    A_w_phi: jax.Array,
    A_wo: jax.Array,
    B_x: jax.Array,
    B_w_gate: jax.Array,
    B_w_up: jax.Array,
    B_w_down: jax.Array,
):
    del B_x
    return pl.pallas_call(
        _kernel,
        out_shape=jax.ShapeDtypeStruct(A_x.shape, A_x.dtype),
        grid=(2,),
        in_specs=[pl.BlockSpec(memory_space=pl.ANY)] * 7,
        out_specs=pl.BlockSpec(memory_space=pl.ANY),
        scratch_shapes=_SCRATCH,
        compiler_params=pltpu.CompilerParams(
            dimension_semantics=("arbitrary",),
            vmem_limit_bytes=100 * 1024 * 1024,
            disable_bounds_checks=True,
            disable_semaphore_checks=True,
        ),
    )(A_x, A_wqkv, jnp.transpose(A_w_phi, (1, 2, 0)), A_wo, B_w_gate, B_w_up, B_w_down)
```

```python
import jax
import jax.numpy as jnp
from jax import lax
import jax.experimental.pallas as pl
import jax.experimental.pallas.tpu as pltpu

S, D, H, DH, F = 2048, 640, 32, 20, 1536
NG = H // 2
EPS = 1e-5
DEN_EPS = 1e-6
LOG2E = 1.4426950408889634
NT = (((1,), (1,)), ((), ()))
f32, bf16 = jnp.float32, jnp.bfloat16

TS = 512
NTILE = S // TS
HX = TS // 2
VA = 256
A0, A1, B1 = 320, 512, 512
NA = 4
OCOLS = (0, 256, 512, 640)
NOC = len(OCOLS) - 1

NFT = 11
KV_W = [(60 * i - 4 * (i % 2), 60 * i - 4 * (i % 2) + 64) for i in range(NFT - 1)] + [(600, 640)]
KV_J = [0 if i % 2 else 60 for i in range(NFT - 1)] + [40]
KV_L = [64] * (NFT - 1) + [48]
KV_OFF = [sum(KV_L[:i]) for i in range(NFT + 1)]

NM, NL = 16 * H, 19 * H
FOLD_H = [(128 * t // DH, (128 * t + 127) // DH) for t in range(5)]
FOLD_M = [(16 * h0, 16 * h1 + 16) for h0, h1 in FOLD_H]
FOLD_T = [(32 * (h0 // 8), 32 * (h1 // 8) + 32) for h0, h1 in FOLD_H]
FOLD_OFF = [sum(m1 - m0 + t1 - t0 for (m0, m1), (t0, t1) in zip(FOLD_M[:i], FOLD_T[:i]))
            for i in range(6)]


def _iota(shape, dim):
    return lax.broadcasted_iota(jnp.int32, shape, dim)


def _dot(a, b):
    return jnp.dot(a, b, preferred_element_type=f32)


def _dot_nt(a, b):
    return lax.dot_general(a, b, NT, preferred_element_type=f32)


def _assemble(parts, ranges, total):
    cuts = sorted({0, total} | {r for rr in ranges for r in rr})
    segs = []
    for a, b in zip(cuts[:-1], cuts[1:]):
        acc = None
        for p, (r0, r1) in zip(parts, ranges):
            if r0 <= a and b <= r1:
                piece = p[a - r0:b - r0]
                acc = piece if acc is None else acc + piece
        segs.append(acc)
    return jnp.concatenate(segs, axis=0)


def _layernorm(x):
    m = jnp.sum(x, axis=-1, keepdims=True) * (1.0 / D)
    xc = x - m
    v = jnp.sum(xc * xc, axis=-1, keepdims=True) * (1.0 / D)
    return xc * lax.rsqrt(v + EPS)


def _gelu(x):
    c = 0.7978845608028654
    return 0.5 * x * (1.0 + jnp.tanh(c * (x + 0.044715 * (x * x * x))))


def _feat(pT, scaled=False):
    ts = pT.shape[1]
    p = pT.reshape(4, 19, 8, ts)
    sub = _iota((4, 8, ts), 1)
    es = [p[:, 0], p[:, 1], p[:, 2], jnp.zeros((4, 8, ts), f32)]
    for d in (1, 2):
        lo = (sub & (2 * d)) == 0
        for i in (0, 2 if d == 1 else 1):
            x, y = es[i], es[i + d]
            es[i] = jnp.where(lo, x, pltpu.roll(y, 2 * d, 1))
            es[i + d] = jnp.where(lo, pltpu.roll(x, 8 - 2 * d, 1), y)
    p = jnp.stack([v for i in range(4) for v in (
        p[:, 3 + 4 * i], p[:, 4 + 4 * i], es[i], p[:, 5 + 4 * i], p[:, 6 + 4 * i])], axis=1)
    p = p.reshape(NG, 5, 8, ts)
    even = _iota((NG, 8, ts), 1) % 2 == 0

    def red(op, x):
        a, b = op(x[:, 0], x[:, 1]), op(x[:, 3], x[:, 4])
        c = op(jnp.where(even, a, b), pltpu.roll(jnp.where(even, b, a), 1, 1))
        c = op(c, x[:, 2])
        c = op(c, pltpu.roll(c, 2, 1))
        return op(c, pltpu.roll(c, 4, 1))

    def spread(c):
        ca, cb = jnp.broadcast_to(c[:, 0:1], c.shape), jnp.broadcast_to(c[:, 1:2], c.shape)
        return jnp.stack([ca, ca, c, cb, cb], axis=1)

    ep = jnp.exp2(p - spread(red(jnp.maximum, p)))
    en = jnp.exp2(spread(red(jnp.minimum, p)) - p)
    sp, rn = red(jnp.add, ep), pl.reciprocal(red(jnp.add, en), approx=True)
    if scaled:
        en = en * spread(rn * sp)
    else:
        ep = ep * spread(pl.reciprocal(sp, approx=True))
        en = en * spread(rn)
    ma = jnp.where(even, ep[:, 2], pltpu.roll(en[:, 2], 1, 1))
    mb = jnp.where(even, pltpu.roll(ep[:, 2], 1, 1), en[:, 2])
    phi = jnp.concatenate([ep[:, 0:2], en[:, 0:2], ma[:, None],
                           ep[:, 3:5], en[:, 3:5], mb[:, None]], axis=1).reshape(2 * D, ts)
    tiles = []
    for i in range(NFT):
        w = phi[120 * i:120 * i + 120]
        tiles.append(jnp.concatenate([w, jnp.zeros((128 - w.shape[0], ts), f32)], axis=0))
    return tiles


def _kernel(x_hbm, wqkv_hbm, wphi_hbm, wo_hbm, wg_hbm, wu_hbm, wd_hbm, o_hbm,
            x_v, wqkv_v, wphi_v, wo_v, wg_v, wu_v, wd_v, out_v,
            wkT, wvT, wqT, perm_s, xn_s, kvT, kv_acc, bdt_s, lhs_s, fq_s, sems, osems):
    n = NTILE

    @pl.when(pl.program_id(0) == 0)
    def _phase1():
        def wblock(r0, nr, c0, s):
            return pltpu.make_async_copy(wqkv_hbm.at[pl.ds(r0, nr), pl.ds(c0, D)],
                                         wqkv_v.at[pl.ds(r0, nr), pl.ds(c0, D)], sems.at[s])

        def xrows(row, nr, s):
            return pltpu.make_async_copy(x_hbm.at[0, pl.ds(row, nr)], x_v.at[pl.ds(row, nr)], sems.at[s])

        def cp_x(t):
            return xrows(pl.multiple_of(t * TS, TS), TS, 10 + t)

        cp_phi = pltpu.make_async_copy(wphi_hbm, wphi_v, sems.at[0])
        cp_x0a, cp_x0b = xrows(0, HX, 9), xrows(HX, HX, 10)
        cp_va, cp_vb = wblock(0, VA, 2 * D, 1), wblock(VA, D - VA, 2 * D, 2)
        cp_k, cp_q = wblock(0, D, D, 3), wblock(0, D, 0, 4)
        cp_ffn = [pltpu.make_async_copy(src, dst, sems.at[5 + j]) for j, (src, dst) in enumerate(
            [(wo_hbm, wo_v), (wg_hbm, wg_v), (wu_hbm, wu_v), (wd_hbm, wd_v)])]
        for c in ([cp_phi, cp_x0a, cp_va, cp_x0b, cp_vb, cp_k, cp_q]
                  + [cp_x(t) for t in range(1, n)] + cp_ffn):
            c.start()

        def put_lhs(t, vT):
            lo = _iota((8, TS), 0) < 4
            for i, (r0, r1) in enumerate(KV_W):
                w = vT[r0:r1]
                if i == NFT - 1:
                    w = jnp.concatenate([w, jnp.ones((8, TS), f32)], axis=0)
                elif i % 2:
                    w = jnp.concatenate([jnp.where(lo, 1.0, w[0:8]), w[8:]], axis=0)
                else:
                    w = jnp.concatenate([w[:56], jnp.where(lo, w[56:64], 1.0)], axis=0)
                lhs_s[t % 2, KV_OFF[i]:KV_OFF[i + 1], :] = w.astype(bf16)

        def put_feat(slot, phi):
            for i in range(NFT):
                fq_s[slot, 128 * i:128 * i + 128, :] = phi[i].astype(bf16)

        def put_kv(kv):
            for i in range(NFT):
                kv_acc[KV_OFF[i]:KV_OFF[i + 1], :] = kv[i]

        def PK(t):
            return _feat(_dot_nt(wkT[...], xn_s[t % 2]))

        def PQ(t):
            put_feat(t, _feat(_dot_nt(wqT[...], xn_s[t % 2]), scaled=True))

        def LNPV(t):
            row = pl.multiple_of(t * TS, TS)
            xn = _layernorm(x_v[pl.ds(row, TS), :].astype(f32)).astype(bf16)
            xn_s[t % 2] = xn
            put_lhs(t, _dot_nt(wvT[...], xn))

        def KV(t, phi):
            return [kv_acc[KV_OFF[i]:KV_OFF[i + 1], :]
                    + _dot_nt(lhs_s[t % 2, KV_OFF[i]:KV_OFF[i + 1], :], phi[i].astype(bf16))
                    for i in range(NFT)]

        def fold(off):
            parts = [_dot_nt(bdt_s[FOLD_OFF[t]:FOLD_OFF[t + 1], :],
                             wqkv_v[:, off + 128 * t:off + 128 * t + 128]) for t in range(5)]
            nm = [m1 - m0 for m0, m1 in FOLD_M]
            wm = _assemble([p[:k] for p, k in zip(parts, nm)], FOLD_M, NM)
            wt = _assemble([p[k:] for p, k in zip(parts, nm)], FOLD_T, 4 * H).reshape(4, 4, 8, D)
            ref = wt[:, 3]
            refm = jnp.concatenate([jnp.broadcast_to(ref[h // 8, h % 8:h % 8 + 1], (16, D))
                                    for h in range(H)], axis=0)
            w = jnp.concatenate([wt[:, :3] - ref[:, None], (wm - refm).reshape(4, 16, 8, D)], axis=1)
            return (w.reshape(NL, D) * LOG2E).astype(bf16)

        kk = _iota((D, 1), 0)
        perm_s[...] = jnp.where(_iota((1, D), 1) == DH * (kk % H) + kk // H, 1.0, 0.0).astype(bf16)
        cp_phi.wait()
        q = jnp.concatenate([wphi_v[d].astype(f32) for d in range(DH)], axis=1).astype(bf16)
        tf = _dot(q, perm_s[...])
        hc = _iota((1, D), 1) // DH
        for t, (h0, h1) in enumerate(FOLD_H):
            tt, ht = tf[:, 128 * t:128 * t + 128], hc[:, 128 * t:128 * t + 128]
            blk = [jnp.where(ht == h, tt[:16], 0.0) for h in range(h0, h1 + 1)]
            for g in range(h0 // 8, h1 // 8 + 1):
                keep = _iota((8, 1), 0) + 8 * g == ht
                blk += [jnp.where(keep, jnp.broadcast_to(tt[16 + k:17 + k], (8, 128)), 0.0)
                        for k in range(4)]
            bdt_s[FOLD_OFF[t]:FOLD_OFF[t + 1], :] = jnp.concatenate(blk, axis=0).astype(bf16)

        def pva(r0, r1, s0, s1):
            return _dot_nt(wvT[r0:r1, 0:VA], xn_s[0, s0:s1, 0:VA])

        def pvb(r0, r1):
            return _dot_nt(wvT[r0:r1, VA:D], xn_s[0, :, VA:D])

        cp_x0a.wait()
        xn_s[0, 0:HX, :] = _layernorm(x_v[0:HX, :].astype(f32)).astype(bf16)
        cp_va.wait()
        wvT[:, 0:VA] = wqkv_v[0:VA, 2 * D:3 * D].T
        paa = pva(0, A0, 0, HX)
        cp_x0b.wait()
        paa = jnp.concatenate([paa, pva(A0, D, 0, HX)], axis=0)
        xn_s[0, HX:TS, :] = _layernorm(x_v[HX:TS, :].astype(f32)).astype(bf16)
        pab = pva(0, A1, HX, TS)
        cp_vb.wait()
        pab = jnp.concatenate([pab, pva(A1, D, HX, TS)], axis=0)
        pa = jnp.concatenate([paa, pab], axis=1)
        wvT[:, VA:D] = wqkv_v[VA:D, 2 * D:3 * D].T
        v0 = pa[0:B1] + pvb(0, B1)
        cp_k.wait()
        wkT[...] = fold(D)
        put_feat(n - 1, PK(0))
        put_lhs(0, jnp.concatenate([v0, pa[B1:D] + pvb(B1, D)], axis=0))
        cp_q.wait()
        cp_x(1).wait()
        wqT[...] = fold(0)
        PQ(0)
        put_kv([_dot_nt(lhs_s[0, KV_OFF[i]:KV_OFF[i + 1], :], fq_s[n - 1, 128 * i:128 * i + 128, :])
                for i in range(NFT)])
        LNPV(1)

        def p1(t, carry):
            cp_x(t + 1).wait()
            fk = PK(t)
            PQ(t)
            kv = KV(t, fk)
            LNPV(t + 1)
            put_kv(kv)
            return carry
        lax.fori_loop(1, n - 1, p1, 0)

        fk = PK(n - 1)
        PQ(n - 1)
        kv = KV(n - 1, fk)
        cc = _iota((1, 128), 1)
        plus_c = jnp.logical_or(cc % 40 < 16, jnp.logical_and(cc % 40 >= 32, cc % 2 == 0))
        eps_c = jnp.where(plus_c, DEN_EPS, 0.0)
        for i, (r0, r1) in enumerate(KV_W):
            j_c = jnp.where(cc < min(120, 2 * D - 120 * i), cc // 40, -64)
            rr = _iota((KV_L[i], 1), 0)
            dlt = rr - (DH * j_c + (60 * i - r0))
            zrow = rr - KV_J[i] == j_c
            keep = jnp.logical_or(jnp.logical_and(dlt >= 0, dlt < DH), zrow)
            kvT[KV_OFF[i]:KV_OFF[i + 1], :] = (jnp.where(keep, kv[i], 0.0)
                                               + jnp.where(zrow, eps_c, 0.0)).astype(bf16)
        for c in cp_ffn:
            c.wait()

    @pl.when(pl.program_id(0) == 1)
    def _phase2():
        def out_copy(t, c):
            row = pl.multiple_of(t * TS, TS)
            c0, c1 = OCOLS[c], OCOLS[c + 1]
            return pltpu.make_async_copy(out_v.at[pl.ds(row, TS), pl.ds(c0, c1 - c0)],
                                         o_hbm.at[0, pl.ds(row, TS), pl.ds(c0, c1 - c0)],
                                         osems.at[t * NOC + c])

        def attn_o(t, c0, c1):
            m = c1 - c0
            parts = [_dot(kvT[KV_OFF[i]:KV_OFF[i + 1], :], fq_s[t, 128 * i:128 * i + 128, c0:c1])
                     for i in range(NFT)]
            sub = _iota((8, m), 0)
            lo = sub < 4
            segs, rds = [], []
            for i in range(0, NFT - 1, 2):
                pe, po = parts[i], parts[i + 1]
                segs += [pe[:56], jnp.where(lo, pe[56:64], po[0:8]), po[8:]]
                rd = 1.0 / jnp.where(sub % 4 == 3, 1.0, jnp.where(lo, po[0:8], pe[56:64]))
                rds += [rd[j:j + 1] for j in (4, 5, 6, 0, 1, 2)]
            segs.append(parts[NFT - 1][:40])
            rd = 1.0 / jnp.where(sub < 2, parts[NFT - 1][40:48], 1.0)
            rds += [rd[0:1], rd[1:2]]
            scale = []
            for g in range(NG):
                a0 = jnp.broadcast_to(rds[2 * g], (8, m))
                a1 = jnp.broadcast_to(rds[2 * g + 1], (8, m))
                scale += [a0, a0, jnp.where(lo, a0, a1), a1, a1]
            return (jnp.concatenate(segs, axis=0) * jnp.concatenate(scale, axis=0)).T.astype(bf16)

        def p2(t, carry):
            row = pl.multiple_of(t * TS, TS)
            ma = TS // NA
            os_ = [attn_o(t, j * ma, (j + 1) * ma) for j in range(NA)]
            hs = [x_v[pl.ds(row + j * ma, ma), :].astype(f32) + _dot(os_[j], wo_v[...]) for j in range(NA)]
            hn = jnp.concatenate([_layernorm(h) for h in hs], axis=0).astype(bf16)
            h = jnp.concatenate(hs, axis=0)
            g = _dot(hn, wg_v[...])
            u = _dot(hn, wu_v[...])
            act = (_gelu(g) * u).astype(bf16)
            for c in range(NOC):
                c0, c1 = OCOLS[c], OCOLS[c + 1]
                out_v[pl.ds(row, TS), c0:c1] = (h[:, c0:c1] + _dot(act, wd_v[:, c0:c1])).astype(bf16)
                out_copy(t, c).start()
            return carry

        lax.fori_loop(0, n, p2, 0)
        for t in range(n):
            for c in range(NOC):
                out_copy(t, c).wait()


_SCRATCH = [
    pltpu.VMEM((S, D), bf16),
    pltpu.VMEM((D, 3 * D), bf16),
    pltpu.VMEM((DH, DH, H), bf16),
    pltpu.VMEM((D, D), bf16),
    pltpu.VMEM((D, F), bf16),
    pltpu.VMEM((D, F), bf16),
    pltpu.VMEM((F, D), bf16),
    pltpu.VMEM((S, D), bf16),
    pltpu.VMEM((NL, D), bf16),
    pltpu.VMEM((D, D), bf16),
    pltpu.VMEM((NL, D), bf16),
    pltpu.VMEM((D, D), bf16),
    pltpu.VMEM((2, TS, D), bf16),
    pltpu.VMEM((KV_OFF[-1], 128), bf16),
    pltpu.VMEM((KV_OFF[-1], 128), f32),
    pltpu.VMEM((FOLD_OFF[-1], 128), bf16),
    pltpu.VMEM((2, KV_OFF[-1], TS), bf16),
    pltpu.VMEM((NTILE, NFT * 128, TS), bf16),
    pltpu.SemaphoreType.DMA((10 + NTILE,)),
    pltpu.SemaphoreType.DMA((NTILE * NOC,)),
]


@jax.jit
def pallas_sequential_preLN__linear_kernel_hedgehog__geglu_ffn__prompt_kernel(
    A_x: jax.Array,
    A_wqkv: jax.Array,
    A_w_phi: jax.Array,
    A_wo: jax.Array,
    B_x: jax.Array,
    B_w_gate: jax.Array,
    B_w_up: jax.Array,
    B_w_down: jax.Array,
):
    del B_x
    return pl.pallas_call(
        _kernel,
        out_shape=jax.ShapeDtypeStruct(A_x.shape, A_x.dtype),
        grid=(2,),
        in_specs=[pl.BlockSpec(memory_space=pl.ANY)] * 7,
        out_specs=pl.BlockSpec(memory_space=pl.ANY),
        scratch_shapes=_SCRATCH,
        compiler_params=pltpu.CompilerParams(
            dimension_semantics=("arbitrary",),
            vmem_limit_bytes=100 * 1024 * 1024,
            disable_bounds_checks=True,
            disable_semaphore_checks=True,
        ),
    )(A_x, A_wqkv, jnp.transpose(A_w_phi, (1, 2, 0)), A_wo, B_w_gate, B_w_up, B_w_down)
```

```python
import jax
import jax.numpy as jnp
from jax import lax
import jax.experimental.pallas as pl
import jax.experimental.pallas.tpu as pltpu

S, D, H, DH, F = 2048, 640, 32, 20, 1536
NG = H // 2
EPS = 1e-5
DEN_EPS = 1e-6
LOG2E = 1.4426950408889634
NT = (((1,), (1,)), ((), ()))
f32, bf16 = jnp.float32, jnp.bfloat16

TS = 512
NTILE = S // TS
HX = TS // 2
VA = 256
A0, A1, B1 = 320, 512, 512
VS = 480
NA = 4
OCH = ((0, 384, 0, 640), (384, 512, 0, 512), (384, 512, 512, 640))
NOC = len(OCH)

NFT = 11
KV_W = [(60 * i - 4 * (i % 2), 60 * i - 4 * (i % 2) + 64) for i in range(NFT - 1)] + [(600, 640)]
KV_J = [0 if i % 2 else 60 for i in range(NFT - 1)] + [40]
KV_L = [64] * (NFT - 1) + [48]
KV_OFF = [sum(KV_L[:i]) for i in range(NFT + 1)]

NM, NL = 16 * H, 19 * H
FOLD_H = [(128 * t // DH, (128 * t + 127) // DH) for t in range(5)]
FOLD_M = [(16 * h0, 16 * h1 + 16) for h0, h1 in FOLD_H]
FOLD_T = [(32 * (h0 // 8), 32 * (h1 // 8) + 32) for h0, h1 in FOLD_H]
FOLD_OFF = [sum(m1 - m0 + t1 - t0 for (m0, m1), (t0, t1) in zip(FOLD_M[:i], FOLD_T[:i]))
            for i in range(6)]


def _iota(shape, dim):
    return lax.broadcasted_iota(jnp.int32, shape, dim)


def _dot(a, b):
    return jnp.dot(a, b, preferred_element_type=f32)


def _dot_nt(a, b):
    return lax.dot_general(a, b, NT, preferred_element_type=f32)


def _assemble(parts, ranges, total):
    cuts = sorted({0, total} | {r for rr in ranges for r in rr})
    segs = []
    for a, b in zip(cuts[:-1], cuts[1:]):
        acc = None
        for p, (r0, r1) in zip(parts, ranges):
            if r0 <= a and b <= r1:
                piece = p[a - r0:b - r0]
                acc = piece if acc is None else acc + piece
        segs.append(acc)
    return jnp.concatenate(segs, axis=0)


def _layernorm(x):
    m = jnp.sum(x, axis=-1, keepdims=True) * (1.0 / D)
    xc = x - m
    v = jnp.sum(xc * xc, axis=-1, keepdims=True) * (1.0 / D)
    return xc * lax.rsqrt(v + EPS)


def _gelu(x):
    c = 0.7978845608028654
    return 0.5 * x * (1.0 + jnp.tanh(c * (x + 0.044715 * (x * x * x))))


def _feat(pT, scaled=False):
    ts = pT.shape[1]
    p = pT.reshape(4, 19, 8, ts)
    sub = _iota((4, 8, ts), 1)
    es = [p[:, 0], p[:, 1], p[:, 2], jnp.zeros((4, 8, ts), f32)]
    for d in (1, 2):
        lo = (sub & (2 * d)) == 0
        for i in (0, 2 if d == 1 else 1):
            x, y = es[i], es[i + d]
            es[i] = jnp.where(lo, x, pltpu.roll(y, 2 * d, 1))
            es[i + d] = jnp.where(lo, pltpu.roll(x, 8 - 2 * d, 1), y)
    p = jnp.stack([v for i in range(4) for v in (
        p[:, 3 + 4 * i], p[:, 4 + 4 * i], es[i], p[:, 5 + 4 * i], p[:, 6 + 4 * i])], axis=1)
    p = p.reshape(NG, 5, 8, ts)
    even = _iota((NG, 8, ts), 1) % 2 == 0

    def red(op, x):
        a, b = op(x[:, 0], x[:, 1]), op(x[:, 3], x[:, 4])
        c = op(jnp.where(even, a, b), pltpu.roll(jnp.where(even, b, a), 1, 1))
        c = op(c, x[:, 2])
        c = op(c, pltpu.roll(c, 2, 1))
        return op(c, pltpu.roll(c, 4, 1))

    def spread(c):
        ca, cb = jnp.broadcast_to(c[:, 0:1], c.shape), jnp.broadcast_to(c[:, 1:2], c.shape)
        return jnp.stack([ca, ca, c, cb, cb], axis=1)

    ep = jnp.exp2(p - spread(red(jnp.maximum, p)))
    en = jnp.exp2(spread(red(jnp.minimum, p)) - p)
    sp, rn = red(jnp.add, ep), pl.reciprocal(red(jnp.add, en), approx=True)
    if scaled:
        en = en * spread(rn * sp)
    else:
        ep = ep * spread(pl.reciprocal(sp, approx=True))
        en = en * spread(rn)
    ma = jnp.where(even, ep[:, 2], pltpu.roll(en[:, 2], 1, 1))
    mb = jnp.where(even, pltpu.roll(ep[:, 2], 1, 1), en[:, 2])
    phi = jnp.concatenate([ep[:, 0:2], en[:, 0:2], ma[:, None],
                           ep[:, 3:5], en[:, 3:5], mb[:, None]], axis=1).reshape(2 * D, ts)
    tiles = []
    for i in range(NFT):
        w = phi[120 * i:120 * i + 120]
        tiles.append(jnp.concatenate([w, jnp.zeros((128 - w.shape[0], ts), f32)], axis=0))
    return tiles


def _kernel(x_hbm, wqkv_hbm, wphi_hbm, wo_hbm, wg_hbm, wu_hbm, wd_hbm, o_hbm,
            x_v, wqkv_v, wphi_v, wo_v, wg_v, wu_v, wd_v, out_v,
            wkT, wvT, wqT, perm_s, xn_s, kvT, kv_acc, bdt_s, lhs_s, fq_s, sems, osems):
    n = NTILE

    @pl.when(pl.program_id(0) == 0)
    def _phase1():
        def wblock(r0, nr, c0, s):
            return pltpu.make_async_copy(wqkv_hbm.at[pl.ds(r0, nr), pl.ds(c0, D)],
                                         wqkv_v.at[pl.ds(r0, nr), pl.ds(c0, D)], sems.at[s])

        def xrows(row, nr, s):
            return pltpu.make_async_copy(x_hbm.at[0, pl.ds(row, nr)], x_v.at[pl.ds(row, nr)], sems.at[s])

        def cp_x(t):
            return xrows(pl.multiple_of(t * TS, TS), TS, 10 + t)

        cp_phi = pltpu.make_async_copy(wphi_hbm, wphi_v, sems.at[0])
        cp_x0a, cp_x0b = xrows(0, HX, 9), xrows(HX, HX, 10)
        cp_va, cp_vb = wblock(0, VA, 2 * D, 1), wblock(VA, D - VA, 2 * D, 2)
        cp_k, cp_q = wblock(0, D, D, 3), wblock(0, D, 0, 4)
        cp_ffn = [pltpu.make_async_copy(src, dst, sems.at[5 + j]) for j, (src, dst) in enumerate(
            [(wo_hbm, wo_v), (wg_hbm, wg_v), (wu_hbm, wu_v), (wd_hbm, wd_v)])]
        for c in ([cp_phi, cp_x0a, cp_va, cp_x0b, cp_vb, cp_k, cp_q]
                  + [cp_x(t) for t in range(1, n)] + cp_ffn):
            c.start()

        def put_lhs(t, vT, base=0):
            lo = _iota((8, TS), 0) < 4
            for i, (r0, r1) in enumerate(KV_W):
                if r0 < base or r1 > base + vT.shape[0]:
                    continue
                w = vT[r0 - base:r1 - base]
                if i == NFT - 1:
                    w = jnp.concatenate([w, jnp.ones((8, TS), f32)], axis=0)
                elif i % 2:
                    w = jnp.concatenate([jnp.where(lo, 1.0, w[0:8]), w[8:]], axis=0)
                else:
                    w = jnp.concatenate([w[:56], jnp.where(lo, w[56:64], 1.0)], axis=0)
                lhs_s[t % 2, KV_OFF[i]:KV_OFF[i + 1], :] = w.astype(bf16)

        def put_feat(slot, phi):
            for i in range(NFT):
                fq_s[slot, 128 * i:128 * i + 128, :] = phi[i].astype(bf16)

        def put_kv(kv):
            for i in range(NFT):
                kv_acc[KV_OFF[i]:KV_OFF[i + 1], :] = kv[i]

        def PK(t):
            return _feat(_dot_nt(wkT[...], xn_s[t % 2]))

        def PQ(t):
            put_feat(t, _feat(_dot_nt(wqT[...], xn_s[t % 2]), scaled=True))

        def LNPV(t):
            row = pl.multiple_of(t * TS, TS)
            xn = _layernorm(x_v[pl.ds(row, TS), :].astype(f32)).astype(bf16)
            xn_s[t % 2] = xn
            put_lhs(t, _dot_nt(wvT[0:VS, :], xn))

        def PVB(t):
            put_lhs(t, _dot_nt(wvT[VS:D, :], xn_s[t % 2]), VS)

        def KV(t, phi):
            return [kv_acc[KV_OFF[i]:KV_OFF[i + 1], :]
                    + _dot_nt(lhs_s[t % 2, KV_OFF[i]:KV_OFF[i + 1], :], phi[i].astype(bf16))
                    for i in range(NFT)]

        def fold(off):
            parts = [_dot_nt(bdt_s[FOLD_OFF[t]:FOLD_OFF[t + 1], :],
                             wqkv_v[:, off + 128 * t:off + 128 * t + 128]) for t in range(5)]
            nm = [m1 - m0 for m0, m1 in FOLD_M]
            wm = _assemble([p[:k] for p, k in zip(parts, nm)], FOLD_M, NM)
            wt = _assemble([p[k:] for p, k in zip(parts, nm)], FOLD_T, 4 * H).reshape(4, 4, 8, D)
            ref = wt[:, 3]
            refm = jnp.concatenate([jnp.broadcast_to(ref[h // 8, h % 8:h % 8 + 1], (16, D))
                                    for h in range(H)], axis=0)
            w = jnp.concatenate([wt[:, :3] - ref[:, None], (wm - refm).reshape(4, 16, 8, D)], axis=1)
            return (w.reshape(NL, D) * LOG2E).astype(bf16)

        kk = _iota((D, 1), 0)
        perm_s[...] = jnp.where(_iota((1, D), 1) == DH * (kk % H) + kk // H, 1.0, 0.0).astype(bf16)
        cp_phi.wait()
        q = jnp.concatenate([wphi_v[d].astype(f32) for d in range(DH)], axis=1).astype(bf16)
        tf = _dot(q, perm_s[...])
        hc = _iota((1, D), 1) // DH
        for t, (h0, h1) in enumerate(FOLD_H):
            tt, ht = tf[:, 128 * t:128 * t + 128], hc[:, 128 * t:128 * t + 128]
            blk = [jnp.where(ht == h, tt[:16], 0.0) for h in range(h0, h1 + 1)]
            for g in range(h0 // 8, h1 // 8 + 1):
                keep = _iota((8, 1), 0) + 8 * g == ht
                blk += [jnp.where(keep, jnp.broadcast_to(tt[16 + k:17 + k], (8, 128)), 0.0)
                        for k in range(4)]
            bdt_s[FOLD_OFF[t]:FOLD_OFF[t + 1], :] = jnp.concatenate(blk, axis=0).astype(bf16)

        def pva(r0, r1, s0, s1):
            return _dot_nt(wvT[r0:r1, 0:VA], xn_s[0, s0:s1, 0:VA])

        def pvb(r0, r1):
            return _dot_nt(wvT[r0:r1, VA:D], xn_s[0, :, VA:D])

        cp_x0a.wait()
        xn_s[0, 0:HX, :] = _layernorm(x_v[0:HX, :].astype(f32)).astype(bf16)
        cp_va.wait()
        wvT[:, 0:VA] = wqkv_v[0:VA, 2 * D:3 * D].T
        paa = pva(0, A0, 0, HX)
        cp_x0b.wait()
        paa = jnp.concatenate([paa, pva(A0, D, 0, HX)], axis=0)
        xn_s[0, HX:TS, :] = _layernorm(x_v[HX:TS, :].astype(f32)).astype(bf16)
        pab = pva(0, A1, HX, TS)
        cp_vb.wait()
        pab = jnp.concatenate([pab, pva(A1, D, HX, TS)], axis=0)
        pa = jnp.concatenate([paa, pab], axis=1)
        wvT[:, VA:D] = wqkv_v[VA:D, 2 * D:3 * D].T
        v0 = pa[0:B1] + pvb(0, B1)
        cp_k.wait()
        wkT[...] = fold(D)
        put_feat(n - 1, PK(0))
        put_lhs(0, jnp.concatenate([v0, pa[B1:D] + pvb(B1, D)], axis=0))
        cp_q.wait()
        cp_x(1).wait()
        wqT[...] = fold(0)
        PQ(0)
        put_kv([_dot_nt(lhs_s[0, KV_OFF[i]:KV_OFF[i + 1], :], fq_s[n - 1, 128 * i:128 * i + 128, :])
                for i in range(NFT)])
        LNPV(1)

        def p1(t, carry):
            cp_x(t + 1).wait()
            fk = PK(t)
            PQ(t)
            PVB(t)
            kv = KV(t, fk)
            LNPV(t + 1)
            put_kv(kv)
            return carry
        lax.fori_loop(1, n - 1, p1, 0)

        fk = PK(n - 1)
        PQ(n - 1)
        PVB(n - 1)
        kv = KV(n - 1, fk)
        cc = _iota((1, 128), 1)
        plus_c = jnp.logical_or(cc % 40 < 16, jnp.logical_and(cc % 40 >= 32, cc % 2 == 0))
        eps_c = jnp.where(plus_c, DEN_EPS, 0.0)
        for i, (r0, r1) in enumerate(KV_W):
            j_c = jnp.where(cc < min(120, 2 * D - 120 * i), cc // 40, -64)
            rr = _iota((KV_L[i], 1), 0)
            dlt = rr - (DH * j_c + (60 * i - r0))
            zrow = rr - KV_J[i] == j_c
            keep = jnp.logical_or(jnp.logical_and(dlt >= 0, dlt < DH), zrow)
            kvT[KV_OFF[i]:KV_OFF[i + 1], :] = (jnp.where(keep, kv[i], 0.0)
                                               + jnp.where(zrow, eps_c, 0.0)).astype(bf16)
        for c in cp_ffn:
            c.wait()

    @pl.when(pl.program_id(0) == 1)
    def _phase2():
        def out_copy(t, c):
            r0, r1, c0, c1 = OCH[c]
            row = pl.multiple_of(t * TS + r0, 128)
            return pltpu.make_async_copy(out_v.at[pl.ds(row, r1 - r0), pl.ds(c0, c1 - c0)],
                                         o_hbm.at[0, pl.ds(row, r1 - r0), pl.ds(c0, c1 - c0)],
                                         osems.at[t * NOC + c])

        def attn_o(t, c0, c1):
            m = c1 - c0
            parts = [_dot(kvT[KV_OFF[i]:KV_OFF[i + 1], :], fq_s[t, 128 * i:128 * i + 128, c0:c1])
                     for i in range(NFT)]
            sub = _iota((8, m), 0)
            lo = sub < 4
            segs, rds = [], []
            for i in range(0, NFT - 1, 2):
                pe, po = parts[i], parts[i + 1]
                segs += [pe[:56], jnp.where(lo, pe[56:64], po[0:8]), po[8:]]
                rd = 1.0 / jnp.where(sub % 4 == 3, 1.0, jnp.where(lo, po[0:8], pe[56:64]))
                rds += [rd[j:j + 1] for j in (4, 5, 6, 0, 1, 2)]
            segs.append(parts[NFT - 1][:40])
            rd = 1.0 / jnp.where(sub < 2, parts[NFT - 1][40:48], 1.0)
            rds += [rd[0:1], rd[1:2]]
            scale = []
            for g in range(NG):
                a0 = jnp.broadcast_to(rds[2 * g], (8, m))
                a1 = jnp.broadcast_to(rds[2 * g + 1], (8, m))
                scale += [a0, a0, jnp.where(lo, a0, a1), a1, a1]
            return (jnp.concatenate(segs, axis=0) * jnp.concatenate(scale, axis=0)).T.astype(bf16)

        def p2(t, carry):
            row = pl.multiple_of(t * TS, TS)
            ma = TS // NA
            os_ = [attn_o(t, j * ma, (j + 1) * ma) for j in range(NA)]
            hs = [x_v[pl.ds(row + j * ma, ma), :].astype(f32) + _dot(os_[j], wo_v[...]) for j in range(NA)]
            hn = jnp.concatenate([_layernorm(h) for h in hs], axis=0).astype(bf16)
            h = jnp.concatenate(hs, axis=0)
            g = _dot(hn, wg_v[...])
            u = _dot(hn, wu_v[...])
            actf = _gelu(g) * u
            acts = {}
            for c, (r0, r1, c0, c1) in enumerate(OCH):
                if (r0, r1) not in acts:
                    acts[(r0, r1)] = actf[r0:r1].astype(bf16)
                out_v[pl.ds(pl.multiple_of(row + r0, 128), r1 - r0), c0:c1] = (
                    h[r0:r1, c0:c1] + _dot(acts[(r0, r1)], wd_v[:, c0:c1])).astype(bf16)
                out_copy(t, c).start()
            return carry

        lax.fori_loop(0, n, p2, 0)
        for t in range(n):
            for c in range(NOC):
                out_copy(t, c).wait()


_SCRATCH = [
    pltpu.VMEM((S, D), bf16),
    pltpu.VMEM((D, 3 * D), bf16),
    pltpu.VMEM((DH, DH, H), bf16),
    pltpu.VMEM((D, D), bf16),
    pltpu.VMEM((D, F), bf16),
    pltpu.VMEM((D, F), bf16),
    pltpu.VMEM((F, D), bf16),
    pltpu.VMEM((S, D), bf16),
    pltpu.VMEM((NL, D), bf16),
    pltpu.VMEM((D, D), bf16),
    pltpu.VMEM((NL, D), bf16),
    pltpu.VMEM((D, D), bf16),
    pltpu.VMEM((2, TS, D), bf16),
    pltpu.VMEM((KV_OFF[-1], 128), bf16),
    pltpu.VMEM((KV_OFF[-1], 128), f32),
    pltpu.VMEM((FOLD_OFF[-1], 128), bf16),
    pltpu.VMEM((2, KV_OFF[-1], TS), bf16),
    pltpu.VMEM((NTILE, NFT * 128, TS), bf16),
    pltpu.SemaphoreType.DMA((10 + NTILE,)),
    pltpu.SemaphoreType.DMA((NTILE * NOC,)),
]


@jax.jit
def pallas_sequential_preLN__linear_kernel_hedgehog__geglu_ffn__prompt_kernel(
    A_x: jax.Array,
    A_wqkv: jax.Array,
    A_w_phi: jax.Array,
    A_wo: jax.Array,
    B_x: jax.Array,
    B_w_gate: jax.Array,
    B_w_up: jax.Array,
    B_w_down: jax.Array,
):
    del B_x
    return pl.pallas_call(
        _kernel,
        out_shape=jax.ShapeDtypeStruct(A_x.shape, A_x.dtype),
        grid=(2,),
        in_specs=[pl.BlockSpec(memory_space=pl.ANY)] * 7,
        out_specs=pl.BlockSpec(memory_space=pl.ANY),
        scratch_shapes=_SCRATCH,
        compiler_params=pltpu.CompilerParams(
            dimension_semantics=("arbitrary",),
            vmem_limit_bytes=100 * 1024 * 1024,
            disable_bounds_checks=True,
            disable_semaphore_checks=True,
        ),
    )(A_x, A_wqkv, jnp.transpose(A_w_phi, (1, 2, 0)), A_wo, B_w_gate, B_w_up, B_w_down)
```

```python
import dataclasses

import jax
import jax.numpy as jnp
from jax import lax
import jax.experimental.pallas as pl
import jax.experimental.pallas.tpu as pltpu

S, D, H, DH, F = 2048, 640, 32, 20, 1536
NG = H // 2
EPS = 1e-5
DEN_EPS = 1e-6
LOG2E = 1.4426950408889634
NT = (((1,), (1,)), ((), ()))
f32, bf16 = jnp.float32, jnp.bfloat16

TS = 512
NTILE = S // TS
HX = TS // 2
VA = 256
A0, A1, B1 = 320, 512, 512
VS = 480
NA = 4
OCH = ((0, 384, 0, 640), (384, 512, 0, 512), (384, 512, 512, 640))
NOC = len(OCH)

NFT = 11
KV_W = [(60 * i - 4 * (i % 2), 60 * i - 4 * (i % 2) + 64) for i in range(NFT - 1)] + [(600, 640)]
KV_J = [0 if i % 2 else 60 for i in range(NFT - 1)] + [40]
KV_L = [64] * (NFT - 1) + [48]
KV_OFF = [sum(KV_L[:i]) for i in range(NFT + 1)]

NM, NL = 16 * H, 19 * H
FOLD_H = [(128 * t // DH, (128 * t + 127) // DH) for t in range(5)]
FOLD_M = [(16 * h0, 16 * h1 + 16) for h0, h1 in FOLD_H]
FOLD_T = [(32 * (h0 // 8), 32 * (h1 // 8) + 32) for h0, h1 in FOLD_H]
FOLD_OFF = [sum(m1 - m0 + t1 - t0 for (m0, m1), (t0, t1) in zip(FOLD_M[:i], FOLD_T[:i]))
            for i in range(6)]


def _iota(shape, dim):
    return lax.broadcasted_iota(jnp.int32, shape, dim)


def _dot(a, b):
    return jnp.dot(a, b, preferred_element_type=f32)


def _dot_nt(a, b):
    return lax.dot_general(a, b, NT, preferred_element_type=f32)


def _assemble(parts, ranges, total):
    cuts = sorted({0, total} | {r for rr in ranges for r in rr})
    segs = []
    for a, b in zip(cuts[:-1], cuts[1:]):
        acc = None
        for p, (r0, r1) in zip(parts, ranges):
            if r0 <= a and b <= r1:
                piece = p[a - r0:b - r0]
                acc = piece if acc is None else acc + piece
        segs.append(acc)
    return jnp.concatenate(segs, axis=0)


def _layernorm(x):
    m = jnp.sum(x, axis=-1, keepdims=True) * (1.0 / D)
    xc = x - m
    v = jnp.sum(xc * xc, axis=-1, keepdims=True) * (1.0 / D)
    return xc * lax.rsqrt(v + EPS)


def _gelu(x):
    c = 0.7978845608028654
    return 0.5 * x * (1.0 + jnp.tanh(c * (x + 0.044715 * (x * x * x))))


def _feat(pT, scaled=False):
    ts = pT.shape[1]
    p = pT.reshape(4, 19, 8, ts)
    sub = _iota((4, 8, ts), 1)
    es = [p[:, 0], p[:, 1], p[:, 2], jnp.zeros((4, 8, ts), f32)]
    for d in (1, 2):
        lo = (sub & (2 * d)) == 0
        for i in (0, 2 if d == 1 else 1):
            x, y = es[i], es[i + d]
            es[i] = jnp.where(lo, x, pltpu.roll(y, 2 * d, 1))
            es[i + d] = jnp.where(lo, pltpu.roll(x, 8 - 2 * d, 1), y)
    p = jnp.stack([v for i in range(4) for v in (
        p[:, 3 + 4 * i], p[:, 4 + 4 * i], es[i], p[:, 5 + 4 * i], p[:, 6 + 4 * i])], axis=1)
    p = p.reshape(NG, 5, 8, ts)
    even = _iota((NG, 8, ts), 1) % 2 == 0

    def red(op, x):
        a, b = op(x[:, 0], x[:, 1]), op(x[:, 3], x[:, 4])
        c = op(jnp.where(even, a, b), pltpu.roll(jnp.where(even, b, a), 1, 1))
        c = op(c, x[:, 2])
        c = op(c, pltpu.roll(c, 2, 1))
        return op(c, pltpu.roll(c, 4, 1))

    def spread(c):
        ca, cb = jnp.broadcast_to(c[:, 0:1], c.shape), jnp.broadcast_to(c[:, 1:2], c.shape)
        return jnp.stack([ca, ca, c, cb, cb], axis=1)

    ep = jnp.exp2(p - spread(red(jnp.maximum, p)))
    en = jnp.exp2(spread(red(jnp.minimum, p)) - p)
    sp, rn = red(jnp.add, ep), pl.reciprocal(red(jnp.add, en), approx=True)
    if scaled:
        en = en * spread(rn * sp)
    else:
        ep = ep * spread(pl.reciprocal(sp, approx=True))
        en = en * spread(rn)
    ma = jnp.where(even, ep[:, 2], pltpu.roll(en[:, 2], 1, 1))
    mb = jnp.where(even, pltpu.roll(ep[:, 2], 1, 1), en[:, 2])
    phi = jnp.concatenate([ep[:, 0:2], en[:, 0:2], ma[:, None],
                           ep[:, 3:5], en[:, 3:5], mb[:, None]], axis=1).reshape(2 * D, ts)
    tiles = []
    for i in range(NFT):
        w = phi[120 * i:120 * i + 120]
        tiles.append(jnp.concatenate([w, jnp.zeros((128 - w.shape[0], ts), f32)], axis=0))
    return tiles


def _kernel(x_hbm, wqkv_hbm, wphi_hbm, wo_hbm, wg_hbm, wu_hbm, wd_hbm, o_hbm,
            x_v, wqkv_v, wphi_v, wo_v, wg_v, wu_v, wd_v, out_v,
            wkT, wvT, wqT, perm_s, xn_s, kvT, kv_acc, bdt_s, lhs_s, fq_s, sems, osems):
    n = NTILE

    @pl.when(pl.program_id(0) == 0)
    def _phase1():
        def wblock(r0, nr, c0, s):
            return pltpu.make_async_copy(wqkv_hbm.at[pl.ds(r0, nr), pl.ds(c0, D)],
                                         wqkv_v.at[pl.ds(r0, nr), pl.ds(c0, D)], sems.at[s])

        def xrows(row, nr, s):
            return pltpu.make_async_copy(x_hbm.at[0, pl.ds(row, nr)], x_v.at[pl.ds(row, nr)], sems.at[s])

        def cp_x(t):
            return xrows(pl.multiple_of(t * TS, TS), TS, 10 + t)

        cp_phi = pltpu.make_async_copy(wphi_hbm, wphi_v, sems.at[0])
        cp_x0a, cp_x0b = xrows(0, HX, 9), xrows(HX, HX, 10)
        cp_va, cp_vb = wblock(0, VA, 2 * D, 1), wblock(VA, D - VA, 2 * D, 2)
        cp_k, cp_q = wblock(0, D, D, 3), wblock(0, D, 0, 4)
        cp_ffn = [pltpu.make_async_copy(src, dst, sems.at[5 + j]) for j, (src, dst) in enumerate(
            [(wo_hbm, wo_v), (wg_hbm, wg_v), (wu_hbm, wu_v), (wd_hbm, wd_v)])]
        for c in ([cp_phi, cp_x0a, cp_va, cp_x0b, cp_vb, cp_k, cp_q]
                  + [cp_x(t) for t in range(1, n)] + cp_ffn):
            c.start()

        def put_lhs(t, vT, base=0):
            lo = _iota((8, TS), 0) < 4
            for i, (r0, r1) in enumerate(KV_W):
                if r0 < base or r1 > base + vT.shape[0]:
                    continue
                w = vT[r0 - base:r1 - base]
                if i == NFT - 1:
                    w = jnp.concatenate([w, jnp.ones((8, TS), f32)], axis=0)
                elif i % 2:
                    w = jnp.concatenate([jnp.where(lo, 1.0, w[0:8]), w[8:]], axis=0)
                else:
                    w = jnp.concatenate([w[:56], jnp.where(lo, w[56:64], 1.0)], axis=0)
                lhs_s[t % 2, KV_OFF[i]:KV_OFF[i + 1], :] = w.astype(bf16)

        def put_feat(slot, phi):
            for i in range(NFT):
                fq_s[slot, 128 * i:128 * i + 128, :] = phi[i].astype(bf16)

        def put_kv(kv):
            for i in range(NFT):
                kv_acc[KV_OFF[i]:KV_OFF[i + 1], :] = kv[i]

        def PK(t):
            return _feat(_dot_nt(wkT[...], xn_s[t % 2]))

        def PQ(t):
            put_feat(t, _feat(_dot_nt(wqT[...], xn_s[t % 2]), scaled=True))

        def LNPV(t):
            row = pl.multiple_of(t * TS, TS)
            xn = _layernorm(x_v[pl.ds(row, TS), :].astype(f32)).astype(bf16)
            xn_s[t % 2] = xn
            put_lhs(t, _dot_nt(wvT[0:VS, :], xn))

        def PVB(t):
            put_lhs(t, _dot_nt(wvT[VS:D, :], xn_s[t % 2]), VS)

        def KV(t, phi):
            return [kv_acc[KV_OFF[i]:KV_OFF[i + 1], :]
                    + _dot_nt(lhs_s[t % 2, KV_OFF[i]:KV_OFF[i + 1], :], phi[i].astype(bf16))
                    for i in range(NFT)]

        def fold(off):
            parts = [_dot_nt(bdt_s[FOLD_OFF[t]:FOLD_OFF[t + 1], :],
                             wqkv_v[:, off + 128 * t:off + 128 * t + 128]) for t in range(5)]
            nm = [m1 - m0 for m0, m1 in FOLD_M]
            wm = _assemble([p[:k] for p, k in zip(parts, nm)], FOLD_M, NM)
            wt = _assemble([p[k:] for p, k in zip(parts, nm)], FOLD_T, 4 * H).reshape(4, 4, 8, D)
            ref = wt[:, 3]
            refm = jnp.concatenate([jnp.broadcast_to(ref[h // 8, h % 8:h % 8 + 1], (16, D))
                                    for h in range(H)], axis=0)
            w = jnp.concatenate([wt[:, :3] - ref[:, None], (wm - refm).reshape(4, 16, 8, D)], axis=1)
            return (w.reshape(NL, D) * LOG2E).astype(bf16)

        kk = _iota((D, 1), 0)
        perm_s[...] = jnp.where(_iota((1, D), 1) == DH * (kk % H) + kk // H, 1.0, 0.0).astype(bf16)
        cp_phi.wait()
        q = jnp.concatenate([wphi_v[d].astype(f32) for d in range(DH)], axis=1).astype(bf16)
        tf = _dot(q, perm_s[...])
        hc = _iota((1, D), 1) // DH
        for t, (h0, h1) in enumerate(FOLD_H):
            tt, ht = tf[:, 128 * t:128 * t + 128], hc[:, 128 * t:128 * t + 128]
            blk = [jnp.where(ht == h, tt[:16], 0.0) for h in range(h0, h1 + 1)]
            for g in range(h0 // 8, h1 // 8 + 1):
                keep = _iota((8, 1), 0) + 8 * g == ht
                blk += [jnp.where(keep, jnp.broadcast_to(tt[16 + k:17 + k], (8, 128)), 0.0)
                        for k in range(4)]
            bdt_s[FOLD_OFF[t]:FOLD_OFF[t + 1], :] = jnp.concatenate(blk, axis=0).astype(bf16)

        def pva(r0, r1, s0, s1):
            return _dot_nt(wvT[r0:r1, 0:VA], xn_s[0, s0:s1, 0:VA])

        def pvb(r0, r1):
            return _dot_nt(wvT[r0:r1, VA:D], xn_s[0, :, VA:D])

        cp_x0a.wait()
        xn_s[0, 0:HX, :] = _layernorm(x_v[0:HX, :].astype(f32)).astype(bf16)
        cp_va.wait()
        wvT[:, 0:VA] = wqkv_v[0:VA, 2 * D:3 * D].T
        paa = pva(0, A0, 0, HX)
        cp_x0b.wait()
        paa = jnp.concatenate([paa, pva(A0, D, 0, HX)], axis=0)
        xn_s[0, HX:TS, :] = _layernorm(x_v[HX:TS, :].astype(f32)).astype(bf16)
        pab = pva(0, A1, HX, TS)
        cp_vb.wait()
        pab = jnp.concatenate([pab, pva(A1, D, HX, TS)], axis=0)
        pa = jnp.concatenate([paa, pab], axis=1)
        wvT[:, VA:D] = wqkv_v[VA:D, 2 * D:3 * D].T
        v0 = pa[0:B1] + pvb(0, B1)
        cp_k.wait()
        wkT[...] = fold(D)
        put_feat(n - 1, PK(0))
        put_lhs(0, jnp.concatenate([v0, pa[B1:D] + pvb(B1, D)], axis=0))
        cp_q.wait()
        cp_x(1).wait()
        wqT[...] = fold(0)
        PQ(0)
        put_kv([_dot_nt(lhs_s[0, KV_OFF[i]:KV_OFF[i + 1], :], fq_s[n - 1, 128 * i:128 * i + 128, :])
                for i in range(NFT)])
        LNPV(1)

        def p1(t, carry):
            cp_x(t + 1).wait()
            fk = PK(t)
            PQ(t)
            PVB(t)
            kv = KV(t, fk)
            LNPV(t + 1)
            put_kv(kv)
            return carry
        lax.fori_loop(1, n - 1, p1, 0)

        fk = PK(n - 1)
        PQ(n - 1)
        PVB(n - 1)
        kv = KV(n - 1, fk)
        cc = _iota((1, 128), 1)
        plus_c = jnp.logical_or(cc % 40 < 16, jnp.logical_and(cc % 40 >= 32, cc % 2 == 0))
        eps_c = jnp.where(plus_c, DEN_EPS, 0.0)
        for i, (r0, r1) in enumerate(KV_W):
            j_c = jnp.where(cc < min(120, 2 * D - 120 * i), cc // 40, -64)
            rr = _iota((KV_L[i], 1), 0)
            dlt = rr - (DH * j_c + (60 * i - r0))
            zrow = rr - KV_J[i] == j_c
            keep = jnp.logical_or(jnp.logical_and(dlt >= 0, dlt < DH), zrow)
            kvT[KV_OFF[i]:KV_OFF[i + 1], :] = (jnp.where(keep, kv[i], 0.0)
                                               + jnp.where(zrow, eps_c, 0.0)).astype(bf16)
        for c in cp_ffn:
            c.wait()

    @pl.when(pl.program_id(0) == 1)
    def _phase2():
        def out_copy(t, c):
            r0, r1, c0, c1 = OCH[c]
            row = pl.multiple_of(t * TS + r0, 128)
            return pltpu.make_async_copy(out_v.at[pl.ds(row, r1 - r0), pl.ds(c0, c1 - c0)],
                                         o_hbm.at[0, pl.ds(row, r1 - r0), pl.ds(c0, c1 - c0)],
                                         osems.at[t * NOC + c])

        def attn_o(t, c0, c1):
            m = c1 - c0
            parts = [_dot(kvT[KV_OFF[i]:KV_OFF[i + 1], :], fq_s[t, 128 * i:128 * i + 128, c0:c1])
                     for i in range(NFT)]
            sub = _iota((8, m), 0)
            lo = sub < 4
            segs, rds = [], []
            for i in range(0, NFT - 1, 2):
                pe, po = parts[i], parts[i + 1]
                segs += [pe[:56], jnp.where(lo, pe[56:64], po[0:8]), po[8:]]
                rd = 1.0 / jnp.where(sub % 4 == 3, 1.0, jnp.where(lo, po[0:8], pe[56:64]))
                rds += [rd[j:j + 1] for j in (4, 5, 6, 0, 1, 2)]
            segs.append(parts[NFT - 1][:40])
            rd = 1.0 / jnp.where(sub < 2, parts[NFT - 1][40:48], 1.0)
            rds += [rd[0:1], rd[1:2]]
            scale = []
            for g in range(NG):
                a0 = jnp.broadcast_to(rds[2 * g], (8, m))
                a1 = jnp.broadcast_to(rds[2 * g + 1], (8, m))
                scale += [a0, a0, jnp.where(lo, a0, a1), a1, a1]
            return (jnp.concatenate(segs, axis=0) * jnp.concatenate(scale, axis=0)).T.astype(bf16)

        def p2(t, carry):
            row = pl.multiple_of(t * TS, TS)
            ma = TS // NA
            os_ = [attn_o(t, j * ma, (j + 1) * ma) for j in range(NA)]
            hs = [x_v[pl.ds(row + j * ma, ma), :].astype(f32) + _dot(os_[j], wo_v[...]) for j in range(NA)]
            hn = jnp.concatenate([_layernorm(h) for h in hs], axis=0).astype(bf16)
            h = jnp.concatenate(hs, axis=0)
            g = _dot(hn, wg_v[...])
            u = _dot(hn, wu_v[...])
            actf = _gelu(g) * u
            acts = {}
            for c, (r0, r1, c0, c1) in enumerate(OCH):
                if (r0, r1) not in acts:
                    acts[(r0, r1)] = actf[r0:r1].astype(bf16)
                out_v[pl.ds(pl.multiple_of(row + r0, 128), r1 - r0), c0:c1] = (
                    h[r0:r1, c0:c1] + _dot(acts[(r0, r1)], wd_v[:, c0:c1])).astype(bf16)
                out_copy(t, c).start()
            return carry

        lax.fori_loop(0, n, p2, 0)
        for t in range(n):
            for c in range(NOC):
                out_copy(t, c).wait()


_SCRATCH = [
    pltpu.VMEM((S, D), bf16),
    pltpu.VMEM((D, 3 * D), bf16),
    pltpu.VMEM((DH, DH, H), bf16),
    pltpu.VMEM((D, D), bf16),
    pltpu.VMEM((D, F), bf16),
    pltpu.VMEM((D, F), bf16),
    pltpu.VMEM((F, D), bf16),
    pltpu.VMEM((S, D), bf16),
    pltpu.VMEM((NL, D), bf16),
    pltpu.VMEM((D, D), bf16),
    pltpu.VMEM((NL, D), bf16),
    pltpu.VMEM((D, D), bf16),
    pltpu.VMEM((2, TS, D), bf16),
    pltpu.VMEM((KV_OFF[-1], 128), bf16),
    pltpu.VMEM((KV_OFF[-1], 128), f32),
    pltpu.VMEM((FOLD_OFF[-1], 128), bf16),
    pltpu.VMEM((2, KV_OFF[-1], TS), bf16),
    pltpu.VMEM((NTILE, NFT * 128, TS), bf16),
    pltpu.SemaphoreType.DMA((10 + NTILE,)),
    pltpu.SemaphoreType.DMA((NTILE * NOC,)),
]


def _compiler_params():
    kw = dict(dimension_semantics=("arbitrary",), vmem_limit_bytes=100 * 1024 * 1024,
              disable_bounds_checks=True, disable_semaphore_checks=True)
    known = {f.name for f in dataclasses.fields(pltpu.CompilerParams)}
    return pltpu.CompilerParams(**{k: v for k, v in kw.items() if k in known})


@jax.jit
def pallas_sequential_preLN__linear_kernel_hedgehog__geglu_ffn__prompt_kernel(
    A_x: jax.Array,
    A_wqkv: jax.Array,
    A_w_phi: jax.Array,
    A_wo: jax.Array,
    B_x: jax.Array,
    B_w_gate: jax.Array,
    B_w_up: jax.Array,
    B_w_down: jax.Array,
):
    del B_x
    return pl.pallas_call(
        _kernel,
        out_shape=jax.ShapeDtypeStruct(A_x.shape, A_x.dtype),
        grid=(2,),
        in_specs=[pl.BlockSpec(memory_space=pl.ANY)] * 7,
        out_specs=pl.BlockSpec(memory_space=pl.ANY),
        scratch_shapes=_SCRATCH,
        compiler_params=_compiler_params(),
    )(A_x, A_wqkv, jnp.transpose(A_w_phi, (1, 2, 0)), A_wo, B_w_gate, B_w_up, B_w_down)
```

```python
import dataclasses

import jax
import jax.numpy as jnp
from jax import lax
import jax.experimental.pallas as pl
import jax.experimental.pallas.tpu as pltpu

S, D, H, DH, F = 2048, 640, 32, 20, 1536
NG = H // 2
FC = 128
SDN = True
NTOP = 2
DC = 128
EPS = 1e-5
DEN_EPS = 1e-6
LOG2E = 1.4426950408889634
NT = (((1,), (1,)), ((), ()))
f32, bf16 = jnp.float32, jnp.bfloat16

TS = 512
NTILE = S // TS
HX = TS // 2
VA = 256
A0, A1, B1 = 320, 512, 512
VS = 480
NA = 4
OCH = ((0, 512, 0, 512), (0, 256, 512, 640), (256, 512, 512, 640))
NOC = len(OCH)

NFT = 11
KV_W = [(60 * i - 4 * (i % 2), 60 * i - 4 * (i % 2) + 64) for i in range(NFT - 1)] + [(600, 640)]
KV_J = [0 if i % 2 else 60 for i in range(NFT - 1)] + [40]
KV_L = [64] * (NFT - 1) + [48]
KV_OFF = [sum(KV_L[:i]) for i in range(NFT + 1)]

NM, NL = 16 * H, 19 * H
FOLD_H = [(128 * t // DH, (128 * t + 127) // DH) for t in range(5)]
FOLD_M = [(16 * h0, 16 * h1 + 16) for h0, h1 in FOLD_H]
FOLD_T = [(32 * (h0 // 8), 32 * (h1 // 8) + 32) for h0, h1 in FOLD_H]
FOLD_OFF = [sum(m1 - m0 + t1 - t0 for (m0, m1), (t0, t1) in zip(FOLD_M[:i], FOLD_T[:i]))
            for i in range(6)]


def _iota(shape, dim):
    return lax.broadcasted_iota(jnp.int32, shape, dim)


def _dot(a, b):
    return jnp.dot(a, b, preferred_element_type=f32)


def _dot_nt(a, b):
    return lax.dot_general(a, b, NT, preferred_element_type=f32)


def _assemble(parts, ranges, total):
    cuts = sorted({0, total} | {r for rr in ranges for r in rr})
    segs = []
    for a, b in zip(cuts[:-1], cuts[1:]):
        acc = None
        for p, (r0, r1) in zip(parts, ranges):
            if r0 <= a and b <= r1:
                piece = p[a - r0:b - r0]
                acc = piece if acc is None else acc + piece
        segs.append(acc)
    return jnp.concatenate(segs, axis=0)


def _layernorm(x):
    m = jnp.sum(x, axis=-1, keepdims=True) * (1.0 / D)
    xc = x - m
    v = jnp.sum(xc * xc, axis=-1, keepdims=True) * (1.0 / D)
    return xc * lax.rsqrt(v + EPS)


def _gelu(x):
    c = 0.7978845608028654
    return 0.5 * x * (1.0 + jnp.tanh(c * (x + 0.044715 * (x * x * x))))


def _strassen_lhs(a11, a12, a21, a22):
    return [x.astype(bf16) for x in (a11 + a22, a21 + a22, a11, a22, a11 + a12, a21 - a11, a12 - a22)]


def _strassen_top(ls, b11, b12, b21, b22):
    m3 = _dot(ls[2], (b12.astype(f32) - b22.astype(f32)).astype(bf16))
    return m3, _dot(ls[4], b22)


def _strassen(ls, b11, b12, b21, b22, top=None):
    m3, m5 = _strassen_top(ls, b11, b12, b21, b22) if top is None else top
    f11, f12, f21, f22 = (b.astype(f32) for b in (b11, b12, b21, b22))
    m1 = _dot(ls[0], (f11 + f22).astype(bf16))
    m4 = _dot(ls[3], (f21 - f11).astype(bf16))
    m7 = _dot(ls[6], (f21 + f22).astype(bf16))
    m2 = _dot(ls[1], b11)
    m6 = _dot(ls[5], (f11 + f12).astype(bf16))
    return m1 + m4 - m5 + m7, m3 + m5, m2 + m4, m1 - m2 + m3 + m6


def _feat(pT, scaled=False):
    ts = pT.shape[1]
    p = pT.reshape(4, 19, 8, ts)
    sub = _iota((4, 8, ts), 1)
    es = [p[:, 0], p[:, 1], p[:, 2], jnp.zeros((4, 8, ts), f32)]
    for d in (1, 2):
        lo = (sub & (2 * d)) == 0
        for i in (0, 2 if d == 1 else 1):
            x, y = es[i], es[i + d]
            es[i] = jnp.where(lo, x, pltpu.roll(y, 2 * d, 1))
            es[i + d] = jnp.where(lo, pltpu.roll(x, 8 - 2 * d, 1), y)
    p = jnp.stack([v for i in range(4) for v in (
        p[:, 3 + 4 * i], p[:, 4 + 4 * i], es[i], p[:, 5 + 4 * i], p[:, 6 + 4 * i])], axis=1)
    p = p.reshape(NG, 5, 8, ts)
    even = _iota((NG, 8, ts), 1) % 2 == 0

    def red(op, x):
        a, b = op(x[:, 0], x[:, 1]), op(x[:, 3], x[:, 4])
        c = op(jnp.where(even, a, b), pltpu.roll(jnp.where(even, b, a), 1, 1))
        c = op(c, x[:, 2])
        c = op(c, pltpu.roll(c, 2, 1))
        return op(c, pltpu.roll(c, 4, 1))

    def spread(c):
        ca, cb = jnp.broadcast_to(c[:, 0:1], c.shape), jnp.broadcast_to(c[:, 1:2], c.shape)
        return jnp.stack([ca, ca, c, cb, cb], axis=1)

    ep = jnp.exp2(p - spread(red(jnp.maximum, p)))
    en = jnp.exp2(spread(red(jnp.minimum, p)) - p)
    sp, rn = red(jnp.add, ep), pl.reciprocal(red(jnp.add, en), approx=True)
    if scaled:
        en = en * spread(rn * sp)
    else:
        ep = ep * spread(pl.reciprocal(sp, approx=True))
        en = en * spread(rn)
    ma = jnp.where(even, ep[:, 2], pltpu.roll(en[:, 2], 1, 1))
    mb = jnp.where(even, pltpu.roll(ep[:, 2], 1, 1), en[:, 2])
    phi = jnp.concatenate([ep[:, 0:2], en[:, 0:2], ma[:, None],
                           ep[:, 3:5], en[:, 3:5], mb[:, None]], axis=1).reshape(2 * D, ts)
    tiles = []
    for i in range(NFT):
        w = phi[120 * i:120 * i + 120]
        tiles.append(jnp.concatenate([w, jnp.zeros((128 - w.shape[0], ts), f32)], axis=0))
    return tiles


def _kernel(x_hbm, wqkv_hbm, wphi_hbm, wo_hbm, wg_hbm, wu_hbm, wd_hbm, o_hbm,
            x_v, wqkv_v, wphi_v, wo_v, wg_v, wu_v, wd_v, out_v,
            wkT, wvT, wqT, perm_s, xn_s, kvT, kv_acc, bdt_s, lhs_s, fq_s, sems, osems):
    n = NTILE

    @pl.when(pl.program_id(0) == 0)
    def _phase1():
        def wblock(r0, nr, c0, s):
            return pltpu.make_async_copy(wqkv_hbm.at[pl.ds(r0, nr), pl.ds(c0, D)],
                                         wqkv_v.at[pl.ds(r0, nr), pl.ds(c0, D)], sems.at[s])

        def xrows(row, nr, s):
            return pltpu.make_async_copy(x_hbm.at[0, pl.ds(row, nr)], x_v.at[pl.ds(row, nr)], sems.at[s])

        def cp_x(t):
            return xrows(pl.multiple_of(t * TS, TS), TS, 10 + t)

        cp_phi = pltpu.make_async_copy(wphi_hbm, wphi_v, sems.at[0])
        cp_x0a, cp_x0b = xrows(0, HX, 9), xrows(HX, HX, 10)
        cp_va, cp_vb = wblock(0, VA, 2 * D, 1), wblock(VA, D - VA, 2 * D, 2)
        cp_k, cp_q = wblock(0, D, D, 3), wblock(0, D, 0, 4)
        cp_ffn = [pltpu.make_async_copy(src, dst, sems.at[5 + j]) for j, (src, dst) in enumerate(
            [(wo_hbm, wo_v), (wg_hbm, wg_v), (wu_hbm, wu_v), (wd_hbm, wd_v)])]
        for c in ([cp_phi, cp_x0a, cp_va, cp_x0b, cp_vb, cp_k, cp_q]
                  + [cp_x(t) for t in range(1, n)] + cp_ffn):
            c.start()

        def put_lhs(t, vT, base=0):
            lo = _iota((8, TS), 0) < 4
            for i, (r0, r1) in enumerate(KV_W):
                if r0 < base or r1 > base + vT.shape[0]:
                    continue
                w = vT[r0 - base:r1 - base]
                if i == NFT - 1:
                    w = jnp.concatenate([w, jnp.ones((8, TS), f32)], axis=0)
                elif i % 2:
                    w = jnp.concatenate([jnp.where(lo, 1.0, w[0:8]), w[8:]], axis=0)
                else:
                    w = jnp.concatenate([w[:56], jnp.where(lo, w[56:64], 1.0)], axis=0)
                lhs_s[t % 2, KV_OFF[i]:KV_OFF[i + 1], :] = w.astype(bf16)

        def put_feat(slot, phi):
            for i in range(NFT):
                fq_s[slot, 128 * i:128 * i + 128, :] = phi[i].astype(bf16)

        def put_kv(kv):
            for i in range(NFT):
                kv_acc[KV_OFF[i]:KV_OFF[i + 1], :] = kv[i]

        def PK(t):
            return _feat(_dot_nt(wkT[...], xn_s[t % 2]))

        def PQ(t):
            put_feat(t, _feat(_dot_nt(wqT[...], xn_s[t % 2]), scaled=True))

        def LNPV(t):
            row = pl.multiple_of(t * TS, TS)
            xn = _layernorm(x_v[pl.ds(row, TS), :].astype(f32)).astype(bf16)
            xn_s[t % 2] = xn
            put_lhs(t, _dot_nt(wvT[0:VS, :], xn))

        def PVB(t):
            put_lhs(t, _dot_nt(wvT[VS:D, :], xn_s[t % 2]), VS)

        def KV(t, phi):
            return [kv_acc[KV_OFF[i]:KV_OFF[i + 1], :]
                    + _dot_nt(lhs_s[t % 2, KV_OFF[i]:KV_OFF[i + 1], :], phi[i].astype(bf16))
                    for i in range(NFT)]

        def fold(off):
            parts = [_dot_nt(bdt_s[FOLD_OFF[t]:FOLD_OFF[t + 1], :],
                             wqkv_v[:, off + 128 * t:off + 128 * t + 128]) for t in range(5)]
            nm = [m1 - m0 for m0, m1 in FOLD_M]
            wm = _assemble([p[:k] for p, k in zip(parts, nm)], FOLD_M, NM)
            wt = _assemble([p[k:] for p, k in zip(parts, nm)], FOLD_T, 4 * H).reshape(4, 4, 8, D)
            ref = wt[:, 3]
            refm = jnp.concatenate([jnp.broadcast_to(ref[h // 8, h % 8:h % 8 + 1], (16, D))
                                    for h in range(H)], axis=0)
            w = jnp.concatenate([wt[:, :3] - ref[:, None], (wm - refm).reshape(4, 16, 8, D)], axis=1)
            return (w.reshape(NL, D) * LOG2E).astype(bf16)

        kk = _iota((D, 1), 0)
        perm_s[...] = jnp.where(_iota((1, D), 1) == DH * (kk % H) + kk // H, 1.0, 0.0).astype(bf16)
        cp_phi.wait()
        q = jnp.concatenate([wphi_v[d].astype(f32) for d in range(DH)], axis=1).astype(bf16)
        tf = _dot(q, perm_s[...])
        hc = _iota((1, D), 1) // DH
        for t, (h0, h1) in enumerate(FOLD_H):
            tt, ht = tf[:, 128 * t:128 * t + 128], hc[:, 128 * t:128 * t + 128]
            blk = [jnp.where(ht == h, tt[:16], 0.0) for h in range(h0, h1 + 1)]
            for g in range(h0 // 8, h1 // 8 + 1):
                keep = _iota((8, 1), 0) + 8 * g == ht
                blk += [jnp.where(keep, jnp.broadcast_to(tt[16 + k:17 + k], (8, 128)), 0.0)
                        for k in range(4)]
            bdt_s[FOLD_OFF[t]:FOLD_OFF[t + 1], :] = jnp.concatenate(blk, axis=0).astype(bf16)

        def pva(r0, r1, s0, s1):
            return _dot_nt(wvT[r0:r1, 0:VA], xn_s[0, s0:s1, 0:VA])

        def pvb(r0, r1):
            return _dot_nt(wvT[r0:r1, VA:D], xn_s[0, :, VA:D])

        cp_x0a.wait()
        xn_s[0, 0:HX, :] = _layernorm(x_v[0:HX, :].astype(f32)).astype(bf16)
        cp_va.wait()
        wvT[:, 0:VA] = wqkv_v[0:VA, 2 * D:3 * D].T
        paa = pva(0, A0, 0, HX)
        cp_x0b.wait()
        paa = jnp.concatenate([paa, pva(A0, D, 0, HX)], axis=0)
        xn_s[0, HX:TS, :] = _layernorm(x_v[HX:TS, :].astype(f32)).astype(bf16)
        pab = pva(0, A1, HX, TS)
        cp_vb.wait()
        pab = jnp.concatenate([pab, pva(A1, D, HX, TS)], axis=0)
        pa = jnp.concatenate([paa, pab], axis=1)
        wvT[:, VA:D] = wqkv_v[VA:D, 2 * D:3 * D].T
        v0 = pa[0:B1] + pvb(0, B1)
        cp_k.wait()
        wkT[...] = fold(D)
        put_feat(n - 1, PK(0))
        put_lhs(0, jnp.concatenate([v0, pa[B1:D] + pvb(B1, D)], axis=0))
        cp_q.wait()
        cp_x(1).wait()
        wqT[...] = fold(0)
        PQ(0)
        put_kv([_dot_nt(lhs_s[0, KV_OFF[i]:KV_OFF[i + 1], :], fq_s[n - 1, 128 * i:128 * i + 128, :])
                for i in range(NFT)])
        LNPV(1)

        def p1(t, carry):
            cp_x(t + 1).wait()
            fk = PK(t)
            PQ(t)
            PVB(t)
            kv = KV(t, fk)
            LNPV(t + 1)
            put_kv(kv)
            return carry
        lax.fori_loop(1, n - 1, p1, 0)

        fk = PK(n - 1)
        PQ(n - 1)
        PVB(n - 1)
        kv = KV(n - 1, fk)
        cc = _iota((1, 128), 1)
        plus_c = jnp.logical_or(cc % 40 < 16, jnp.logical_and(cc % 40 >= 32, cc % 2 == 0))
        eps_c = jnp.where(plus_c, DEN_EPS, 0.0)
        for i, (r0, r1) in enumerate(KV_W):
            j_c = jnp.where(cc < min(120, 2 * D - 120 * i), cc // 40, -64)
            rr = _iota((KV_L[i], 1), 0)
            dlt = rr - (DH * j_c + (60 * i - r0))
            zrow = rr - KV_J[i] == j_c
            keep = jnp.logical_or(jnp.logical_and(dlt >= 0, dlt < DH), zrow)
            kvT[KV_OFF[i]:KV_OFF[i + 1], :] = (jnp.where(keep, kv[i], 0.0)
                                               + jnp.where(zrow, eps_c, 0.0)).astype(bf16)
        for c in cp_ffn:
            c.wait()

    @pl.when(pl.program_id(0) == 1)
    def _phase2():
        def out_copy(t, c):
            r0, r1, c0, c1 = OCH[c]
            row = pl.multiple_of(t * TS + r0, 128)
            return pltpu.make_async_copy(out_v.at[pl.ds(row, r1 - r0), pl.ds(c0, c1 - c0)],
                                         o_hbm.at[0, pl.ds(row, r1 - r0), pl.ds(c0, c1 - c0)],
                                         osems.at[t * NOC + c])

        def attn_o(t, c0, c1):
            m = c1 - c0
            parts = [_dot(kvT[KV_OFF[i]:KV_OFF[i + 1], :], fq_s[t, 128 * i:128 * i + 128, c0:c1])
                     for i in range(NFT)]
            sub = _iota((8, m), 0)
            lo = sub < 4
            segs, rds = [], []
            for i in range(0, NFT - 1, 2):
                pe, po = parts[i], parts[i + 1]
                segs += [pe[:56], jnp.where(lo, pe[56:64], po[0:8]), po[8:]]
                rd = 1.0 / jnp.where(sub % 4 == 3, 1.0, jnp.where(lo, po[0:8], pe[56:64]))
                rds += [rd[j:j + 1] for j in (4, 5, 6, 0, 1, 2)]
            segs.append(parts[NFT - 1][:40])
            rd = 1.0 / jnp.where(sub < 2, parts[NFT - 1][40:48], 1.0)
            rds += [rd[0:1], rd[1:2]]
            scale = []
            for g in range(NG):
                a0 = jnp.broadcast_to(rds[2 * g], (8, m))
                a1 = jnp.broadcast_to(rds[2 * g + 1], (8, m))
                scale += [a0, a0, jnp.where(lo, a0, a1), a1, a1]
            return (jnp.concatenate(segs, axis=0) * jnp.concatenate(scale, axis=0)).T.astype(bf16)

        def p2(t, carry):
            row = pl.multiple_of(t * TS, TS)
            ma = TS // NA
            os_ = [attn_o(t, j * ma, (j + 1) * ma) for j in range(NA)]
            hs = [x_v[pl.ds(row + j * ma, ma), :].astype(f32) + _dot(os_[j], wo_v[...]) for j in range(NA)]
            hn = jnp.concatenate([_layernorm(h) for h in hs], axis=0)
            h = jnp.concatenate(hs, axis=0)
            ls = _strassen_lhs(hn[:HX, 0:256], hn[:HX, 256:512], hn[HX:, 0:256], hn[HX:, 256:512])
            hr = hn[:, 512:D].astype(bf16)
            FH = F // 2

            def blocks(w, c0):
                c1 = c0 + FC
                return (w[0:256, c0:c1], w[0:256, FH + c0:FH + c1],
                        w[256:512, c0:c1], w[256:512, FH + c0:FH + c1])

            def proj(w, c0, top):
                c1 = c0 + FC
                c11, c12, c21, c22 = _strassen(ls, *blocks(w, c0), top=top)
                left = jnp.concatenate([c11, c21], axis=0) + _dot(hr, w[512:D, c0:c1])
                right = jnp.concatenate([c12, c22], axis=0) + _dot(hr, w[512:D, FH + c0:FH + c1])
                return left, right

            tops = {}
            for c0 in range(0, NTOP * FC, FC):
                tops['g', c0] = _strassen_top(ls, *blocks(wg_v, c0))
                tops['u', c0] = _strassen_top(ls, *blocks(wu_v, c0))
            al, ar = [], []
            for c0 in range(0, FH, FC):
                gl, gr = proj(wg_v, c0, tops.get(('g', c0)))
                ul, ur = proj(wu_v, c0, tops.get(('u', c0)))
                al.append(_gelu(gl) * ul)
                ar.append(_gelu(gr) * ur)
            al, ar = jnp.concatenate(al, axis=1), jnp.concatenate(ar, axis=1)
            if SDN:
                la = _strassen_lhs(al[:HX], ar[:HX], al[HX:], ar[HX:])
                for c0 in range(0, 256, DC):
                    c1 = c0 + DC
                    c11, c12, c21, c22 = _strassen(la, wd_v[0:FH, c0:c1], wd_v[0:FH, 256 + c0:256 + c1],
                                                   wd_v[FH:F, c0:c1], wd_v[FH:F, 256 + c0:256 + c1])
                    out_v[pl.ds(row, TS), c0:c1] = (
                        h[:, c0:c1] + jnp.concatenate([c11, c21], axis=0)).astype(bf16)
                    out_v[pl.ds(row, TS), 256 + c0:256 + c1] = (
                        h[:, 256 + c0:256 + c1] + jnp.concatenate([c12, c22], axis=0)).astype(bf16)
                out_copy(t, 0).start()
                top = _dot(la[2], wd_v[0:FH, 512:D]) + _dot(ar[:HX].astype(bf16), wd_v[FH:F, 512:D])
                out_v[pl.ds(row, HX), 512:D] = (h[:HX, 512:D] + top).astype(bf16)
                out_copy(t, 1).start()
                bot = _dot(al[HX:].astype(bf16), wd_v[0:FH, 512:D]) + _dot(la[3], wd_v[FH:F, 512:D])
                out_v[pl.ds(pl.multiple_of(row + HX, 128), HX), 512:D] = (h[HX:, 512:D] + bot).astype(bf16)
                out_copy(t, 2).start()
            else:
                actf = jnp.concatenate([al, ar], axis=1)
                acts = {}
                for c, (r0, r1, c0, c1) in enumerate(OCH):
                    if (r0, r1) not in acts:
                        acts[(r0, r1)] = actf[r0:r1].astype(bf16)
                    out_v[pl.ds(pl.multiple_of(row + r0, 128), r1 - r0), c0:c1] = (
                        h[r0:r1, c0:c1] + _dot(acts[(r0, r1)], wd_v[:, c0:c1])).astype(bf16)
                    out_copy(t, c).start()
            return carry

        lax.fori_loop(0, n, p2, 0)
        for t in range(n):
            for c in range(NOC):
                out_copy(t, c).wait()


_SCRATCH = [
    pltpu.VMEM((S, D), bf16),
    pltpu.VMEM((D, 3 * D), bf16),
    pltpu.VMEM((DH, DH, H), bf16),
    pltpu.VMEM((D, D), bf16),
    pltpu.VMEM((D, F), bf16),
    pltpu.VMEM((D, F), bf16),
    pltpu.VMEM((F, D), bf16),
    pltpu.VMEM((S, D), bf16),
    pltpu.VMEM((NL, D), bf16),
    pltpu.VMEM((D, D), bf16),
    pltpu.VMEM((NL, D), bf16),
    pltpu.VMEM((D, D), bf16),
    pltpu.VMEM((2, TS, D), bf16),
    pltpu.VMEM((KV_OFF[-1], 128), bf16),
    pltpu.VMEM((KV_OFF[-1], 128), f32),
    pltpu.VMEM((FOLD_OFF[-1], 128), bf16),
    pltpu.VMEM((2, KV_OFF[-1], TS), bf16),
    pltpu.VMEM((NTILE, NFT * 128, TS), bf16),
    pltpu.SemaphoreType.DMA((10 + NTILE,)),
    pltpu.SemaphoreType.DMA((NTILE * NOC,)),
]


def _compiler_params():
    kw = dict(dimension_semantics=("arbitrary",), vmem_limit_bytes=100 * 1024 * 1024,
              disable_bounds_checks=True, disable_semaphore_checks=True)
    known = {f.name for f in dataclasses.fields(pltpu.CompilerParams)}
    return pltpu.CompilerParams(**{k: v for k, v in kw.items() if k in known})


@jax.jit
def pallas_sequential_preLN__linear_kernel_hedgehog__geglu_ffn__prompt_kernel(
    A_x: jax.Array,
    A_wqkv: jax.Array,
    A_w_phi: jax.Array,
    A_wo: jax.Array,
    B_x: jax.Array,
    B_w_gate: jax.Array,
    B_w_up: jax.Array,
    B_w_down: jax.Array,
):
    del B_x
    return pl.pallas_call(
        _kernel,
        out_shape=jax.ShapeDtypeStruct(A_x.shape, A_x.dtype),
        grid=(2,),
        in_specs=[pl.BlockSpec(memory_space=pl.ANY)] * 7,
        out_specs=pl.BlockSpec(memory_space=pl.ANY),
        scratch_shapes=_SCRATCH,
        compiler_params=_compiler_params(),
    )(A_x, A_wqkv, jnp.transpose(A_w_phi, (1, 2, 0)), A_wo, B_w_gate, B_w_up, B_w_down)
```

```python
import dataclasses

import jax
import jax.numpy as jnp
from jax import lax
import jax.experimental.pallas as pl
import jax.experimental.pallas.tpu as pltpu

S, D, H, DH, F = 2048, 640, 32, 20, 1536
NG = H // 2
EPS = 1e-5
DEN_EPS = 1e-6
LOG2E = 1.4426950408889634
NT = (((1,), (1,)), ((), ()))
f32, bf16 = jnp.float32, jnp.bfloat16

TS = 512
NTILE = S // TS
HX = TS // 2
VA = 256
A0, A1, B1 = 320, 512, 512
VS = 480
NA = 4
WR = 64
OCH = ((0, TS, 0, 512), (0, HX, 512, D), (HX, TS, 512, D))
NOC = len(OCH)

NFT = 11
KV_W = [(60 * i - 4 * (i % 2), 60 * i - 4 * (i % 2) + 64) for i in range(NFT - 1)] + [(600, 640)]
KV_J = [0 if i % 2 else 60 for i in range(NFT - 1)] + [40]
KV_L = [64] * (NFT - 1) + [48]
KV_OFF = [sum(KV_L[:i]) for i in range(NFT + 1)]

NM, NL = 16 * H, 19 * H
FOLD_H = [(128 * t // DH, (128 * t + 127) // DH) for t in range(5)]
FOLD_M = [(16 * h0, 16 * h1 + 16) for h0, h1 in FOLD_H]
FOLD_T = [(32 * (h0 // 8), 32 * (h1 // 8) + 32) for h0, h1 in FOLD_H]
FOLD_OFF = [sum(m1 - m0 + t1 - t0 for (m0, m1), (t0, t1) in zip(FOLD_M[:i], FOLD_T[:i]))
            for i in range(6)]


def _iota(shape, dim):
    return lax.broadcasted_iota(jnp.int32, shape, dim)


def _dot(a, b):
    return jnp.dot(a, b, preferred_element_type=f32)


def _dot_nt(a, b):
    return lax.dot_general(a, b, NT, preferred_element_type=f32)


def _assemble(parts, ranges, total):
    cuts = sorted({0, total} | {r for rr in ranges for r in rr})
    segs = []
    for a, b in zip(cuts[:-1], cuts[1:]):
        acc = None
        for p, (r0, r1) in zip(parts, ranges):
            if r0 <= a and b <= r1:
                piece = p[a - r0:b - r0]
                acc = piece if acc is None else acc + piece
        segs.append(acc)
    return jnp.concatenate(segs, axis=0)


def _layernorm(x):
    m = jnp.sum(x, axis=-1, keepdims=True) * (1.0 / D)
    xc = x - m
    v = jnp.sum(xc * xc, axis=-1, keepdims=True) * (1.0 / D)
    return xc * lax.rsqrt(v + EPS)


def _gelu(x):
    c = 0.7978845608028654
    return 0.5 * x * (1.0 + jnp.tanh(c * (x + 0.044715 * (x * x * x))))


def _strassen_lhs(a11, a12, a21, a22):
    return [x.astype(bf16) for x in (a11 + a22, a21 + a22, a11, a22, a11 + a12, a21 - a11, a12 - a22)]


def _strassen(la, b11, b12, b21, b22):
    f11, f12, f21, f22 = (b.astype(f32) for b in (b11, b12, b21, b22))
    m3 = _dot(la[2], (f12 - f22).astype(bf16))
    m5 = _dot(la[4], b22)
    c12 = m3 + m5
    m1 = _dot(la[0], (f11 + f22).astype(bf16))
    c11, c22 = m1 - m5, m1 + m3
    m4 = _dot(la[3], (f21 - f11).astype(bf16))
    c11 = c11 + m4
    c11 = c11 + _dot(la[6], (f21 + f22).astype(bf16))
    m2 = _dot(la[1], b11)
    c21, c22 = m2 + m4, c22 - m2
    c22 = c22 + _dot(la[5], (f11 + f12).astype(bf16))
    return jnp.concatenate([c11, c21], axis=0), jnp.concatenate([c12, c22], axis=0)


def _feat(pT, scaled=False):
    ts = pT.shape[1]
    p = pT.reshape(4, 19, 8, ts)
    sub = _iota((4, 8, ts), 1)
    es = [p[:, 0], p[:, 1], p[:, 2], jnp.zeros((4, 8, ts), f32)]
    for d in (1, 2):
        lo = (sub & (2 * d)) == 0
        for i in (0, 2 if d == 1 else 1):
            x, y = es[i], es[i + d]
            es[i] = jnp.where(lo, x, pltpu.roll(y, 2 * d, 1))
            es[i + d] = jnp.where(lo, pltpu.roll(x, 8 - 2 * d, 1), y)
    p = jnp.stack([v for i in range(4) for v in (
        p[:, 3 + 4 * i], p[:, 4 + 4 * i], es[i], p[:, 5 + 4 * i], p[:, 6 + 4 * i])], axis=1)
    p = p.reshape(NG, 5, 8, ts)
    even = _iota((NG, 8, ts), 1) % 2 == 0

    def red(op, x):
        a, b = op(x[:, 0], x[:, 1]), op(x[:, 3], x[:, 4])
        c = op(jnp.where(even, a, b), pltpu.roll(jnp.where(even, b, a), 1, 1))
        c = op(c, x[:, 2])
        c = op(c, pltpu.roll(c, 2, 1))
        return op(c, pltpu.roll(c, 4, 1))

    def spread(c):
        ca, cb = jnp.broadcast_to(c[:, 0:1], c.shape), jnp.broadcast_to(c[:, 1:2], c.shape)
        return jnp.stack([ca, ca, c, cb, cb], axis=1)

    ep = jnp.exp2(p - spread(red(jnp.maximum, p)))
    en = jnp.exp2(spread(red(jnp.minimum, p)) - p)
    sp, rn = red(jnp.add, ep), pl.reciprocal(red(jnp.add, en), approx=True)
    if scaled:
        en = en * spread(rn * sp)
    else:
        ep = ep * spread(pl.reciprocal(sp, approx=True))
        en = en * spread(rn)
    ma = jnp.where(even, ep[:, 2], pltpu.roll(en[:, 2], 1, 1))
    mb = jnp.where(even, pltpu.roll(ep[:, 2], 1, 1), en[:, 2])
    phi = jnp.concatenate([ep[:, 0:2], en[:, 0:2], ma[:, None],
                           ep[:, 3:5], en[:, 3:5], mb[:, None]], axis=1).reshape(2 * D, ts)
    tiles = []
    for i in range(NFT):
        w = phi[120 * i:120 * i + 120]
        tiles.append(jnp.concatenate([w, jnp.zeros((128 - w.shape[0], ts), f32)], axis=0))
    return tiles


def _kernel(x_hbm, wqkv_hbm, wphi_hbm, wo_hbm, wg_hbm, wu_hbm, wd_hbm, o_hbm,
            x_v, wqkv_v, wphi_v, wo_v, wg_v, wu_v, wd_v, out_v,
            wkT, wvT, wqT, perm_s, xn_s, kvT, kv_acc, bdt_s, lhs_s, fq_s, sems, osems):
    n = NTILE

    @pl.when(pl.program_id(0) == 0)
    def _phase1():
        def wblock(r0, nr, c0, s):
            return pltpu.make_async_copy(wqkv_hbm.at[pl.ds(r0, nr), pl.ds(c0, D)],
                                         wqkv_v.at[pl.ds(r0, nr), pl.ds(c0, D)], sems.at[s])

        def xrows(row, nr, s):
            return pltpu.make_async_copy(x_hbm.at[0, pl.ds(row, nr)], x_v.at[pl.ds(row, nr)], sems.at[s])

        def cp_x(t):
            return xrows(pl.multiple_of(t * TS, TS), TS, 10 + t)

        cp_phi = pltpu.make_async_copy(wphi_hbm, wphi_v, sems.at[0])
        cp_x0a, cp_x0b = xrows(0, HX, 9), xrows(HX, HX, 10)
        cp_va, cp_vb = wblock(0, VA, 2 * D, 1), wblock(VA, D - VA, 2 * D, 2)
        cp_k, cp_q = wblock(0, D, D, 3), wblock(0, D, 0, 4)
        cp_ffn = [pltpu.make_async_copy(src, dst, sems.at[5 + j]) for j, (src, dst) in enumerate(
            [(wo_hbm, wo_v), (wg_hbm, wg_v), (wu_hbm, wu_v), (wd_hbm, wd_v)])]
        for c in ([cp_phi, cp_x0a, cp_va, cp_x0b, cp_vb, cp_k, cp_q]
                  + [cp_x(t) for t in range(1, n)] + cp_ffn):
            c.start()

        def put_lhs(t, vT, base=0):
            lo = _iota((8, TS), 0) < 4
            for i, (r0, r1) in enumerate(KV_W):
                if r0 < base or r1 > base + vT.shape[0]:
                    continue
                w = vT[r0 - base:r1 - base]
                if i == NFT - 1:
                    w = jnp.concatenate([w, jnp.ones((8, TS), f32)], axis=0)
                elif i % 2:
                    w = jnp.concatenate([jnp.where(lo, 1.0, w[0:8]), w[8:]], axis=0)
                else:
                    w = jnp.concatenate([w[:56], jnp.where(lo, w[56:64], 1.0)], axis=0)
                lhs_s[t % 2, KV_OFF[i]:KV_OFF[i + 1], :] = w.astype(bf16)

        def put_feat(slot, phi):
            for i in range(NFT):
                fq_s[slot, 128 * i:128 * i + 128, :] = phi[i].astype(bf16)

        def put_kv(kv):
            for i in range(NFT):
                kv_acc[KV_OFF[i]:KV_OFF[i + 1], :] = kv[i]

        def PK(t):
            return _feat(_dot_nt(wkT[...], xn_s[t % 2]))

        def PQ(t):
            put_feat(t, _feat(_dot_nt(wqT[...], xn_s[t % 2]), scaled=True))

        def LNPV(t):
            row = pl.multiple_of(t * TS, TS)
            xn = _layernorm(x_v[pl.ds(row, TS), :].astype(f32)).astype(bf16)
            xn_s[t % 2] = xn
            put_lhs(t, _dot_nt(wvT[0:VS, :], xn))

        def PVB(t):
            put_lhs(t, _dot_nt(wvT[VS:D, :], xn_s[t % 2]), VS)

        def KV(t, phi):
            return [kv_acc[KV_OFF[i]:KV_OFF[i + 1], :]
                    + _dot_nt(lhs_s[t % 2, KV_OFF[i]:KV_OFF[i + 1], :], phi[i].astype(bf16))
                    for i in range(NFT)]

        def fold(off):
            parts = [_dot_nt(bdt_s[FOLD_OFF[t]:FOLD_OFF[t + 1], :],
                             wqkv_v[:, off + 128 * t:off + 128 * t + 128]) for t in range(5)]
            nm = [m1 - m0 for m0, m1 in FOLD_M]
            wm = _assemble([p[:k] for p, k in zip(parts, nm)], FOLD_M, NM)
            wt = _assemble([p[k:] for p, k in zip(parts, nm)], FOLD_T, 4 * H).reshape(4, 4, 8, D)
            ref = wt[:, 3]
            refm = jnp.concatenate([jnp.broadcast_to(ref[h // 8, h % 8:h % 8 + 1], (16, D))
                                    for h in range(H)], axis=0)
            w = jnp.concatenate([wt[:, :3] - ref[:, None], (wm - refm).reshape(4, 16, 8, D)], axis=1)
            return (w.reshape(NL, D) * LOG2E).astype(bf16)

        kk = _iota((D, 1), 0)
        perm_s[...] = jnp.where(_iota((1, D), 1) == DH * (kk % H) + kk // H, 1.0, 0.0).astype(bf16)
        cp_phi.wait()
        q = jnp.concatenate([wphi_v[d].astype(f32) for d in range(DH)], axis=1).astype(bf16)
        tf = _dot(q, perm_s[...])
        hc = _iota((1, D), 1) // DH
        for t, (h0, h1) in enumerate(FOLD_H):
            tt, ht = tf[:, 128 * t:128 * t + 128], hc[:, 128 * t:128 * t + 128]
            blk = [jnp.where(ht == h, tt[:16], 0.0) for h in range(h0, h1 + 1)]
            for g in range(h0 // 8, h1 // 8 + 1):
                keep = _iota((8, 1), 0) + 8 * g == ht
                blk += [jnp.where(keep, jnp.broadcast_to(tt[16 + k:17 + k], (8, 128)), 0.0)
                        for k in range(4)]
            bdt_s[FOLD_OFF[t]:FOLD_OFF[t + 1], :] = jnp.concatenate(blk, axis=0).astype(bf16)

        def pva(r0, r1, s0, s1):
            return _dot_nt(wvT[r0:r1, 0:VA], xn_s[0, s0:s1, 0:VA])

        def pvb(r0, r1):
            return _dot_nt(wvT[r0:r1, VA:D], xn_s[0, :, VA:D])

        cp_x0a.wait()
        xn_s[0, 0:HX, :] = _layernorm(x_v[0:HX, :].astype(f32)).astype(bf16)
        cp_va.wait()
        wvT[:, 0:VA] = wqkv_v[0:VA, 2 * D:3 * D].T
        paa = pva(0, A0, 0, HX)
        cp_x0b.wait()
        paa = jnp.concatenate([paa, pva(A0, D, 0, HX)], axis=0)
        xn_s[0, HX:TS, :] = _layernorm(x_v[HX:TS, :].astype(f32)).astype(bf16)
        pab = pva(0, A1, HX, TS)
        cp_vb.wait()
        pab = jnp.concatenate([pab, pva(A1, D, HX, TS)], axis=0)
        pa = jnp.concatenate([paa, pab], axis=1)
        wvT[:, VA:D] = wqkv_v[VA:D, 2 * D:3 * D].T
        v0 = pa[0:B1] + pvb(0, B1)
        cp_k.wait()
        wkT[...] = fold(D)
        put_feat(n - 1, PK(0))
        put_lhs(0, jnp.concatenate([v0, pa[B1:D] + pvb(B1, D)], axis=0))
        cp_q.wait()
        cp_x(1).wait()
        wqT[...] = fold(0)
        PQ(0)
        put_kv([_dot_nt(lhs_s[0, KV_OFF[i]:KV_OFF[i + 1], :], fq_s[n - 1, 128 * i:128 * i + 128, :])
                for i in range(NFT)])
        LNPV(1)

        def p1(t, carry):
            cp_x(t + 1).wait()
            fk = PK(t)
            PQ(t)
            PVB(t)
            kv = KV(t, fk)
            LNPV(t + 1)
            put_kv(kv)
            return carry
        lax.fori_loop(1, n - 1, p1, 0)

        fk = PK(n - 1)
        PQ(n - 1)
        PVB(n - 1)
        kv = KV(n - 1, fk)
        cc = _iota((1, 128), 1)
        plus_c = jnp.logical_or(cc % 40 < 16, jnp.logical_and(cc % 40 >= 32, cc % 2 == 0))
        eps_c = jnp.where(plus_c, DEN_EPS, 0.0)
        for i, (r0, r1) in enumerate(KV_W):
            j_c = jnp.where(cc < min(120, 2 * D - 120 * i), cc // 40, -64)
            rr = _iota((KV_L[i], 1), 0)
            dlt = rr - (DH * j_c + (60 * i - r0))
            zrow = rr - KV_J[i] == j_c
            keep = jnp.logical_or(jnp.logical_and(dlt >= 0, dlt < DH), zrow)
            kvT[KV_OFF[i]:KV_OFF[i + 1], :] = (jnp.where(keep, kv[i], 0.0)
                                               + jnp.where(zrow, eps_c, 0.0)).astype(bf16)
        for c in cp_ffn:
            c.wait()

    @pl.when(pl.program_id(0) == 1)
    def _phase2():
        def out_copy(t, c):
            r0, r1, c0, c1 = OCH[c]
            row = pl.multiple_of(t * TS + r0, 128)
            return pltpu.make_async_copy(out_v.at[pl.ds(row, r1 - r0), pl.ds(c0, c1 - c0)],
                                         o_hbm.at[0, pl.ds(row, r1 - r0), pl.ds(c0, c1 - c0)],
                                         osems.at[t * NOC + c])

        def attn_o(t, c0, c1):
            m = c1 - c0
            parts = [_dot(kvT[KV_OFF[i]:KV_OFF[i + 1], :], fq_s[t, 128 * i:128 * i + 128, c0:c1])
                     for i in range(NFT)]
            sub = _iota((8, m), 0)
            lo = sub < 4
            segs, rds = [], []
            for i in range(0, NFT - 1, 2):
                pe, po = parts[i], parts[i + 1]
                segs += [pe[:56], jnp.where(lo, pe[56:64], po[0:8]), po[8:]]
                rd = 1.0 / jnp.where(sub % 4 == 3, 1.0, jnp.where(lo, po[0:8], pe[56:64]))
                rds += [rd[j:j + 1] for j in (4, 5, 6, 0, 1, 2)]
            segs.append(parts[NFT - 1][:40])
            rd = 1.0 / jnp.where(sub < 2, parts[NFT - 1][40:48], 1.0)
            rds += [rd[0:1], rd[1:2]]
            scale = []
            for g in range(NG):
                a0 = jnp.broadcast_to(rds[2 * g], (8, m))
                a1 = jnp.broadcast_to(rds[2 * g + 1], (8, m))
                scale += [a0, a0, jnp.where(lo, a0, a1), a1, a1]
            return (jnp.concatenate(segs, axis=0) * jnp.concatenate(scale, axis=0)).T

        def p2(t, carry):
            row = pl.multiple_of(t * TS, TS)
            ma = TS // NA
            o = jnp.concatenate([attn_o(t, j * ma, (j + 1) * ma) for j in range(NA)], axis=0)
            hs = [x_v[pl.ds(row + r0, WR), :].astype(f32) + _dot(o[r0:r0 + WR].astype(bf16), wo_v[...])
                  for r0 in range(0, TS, WR)]
            hn = jnp.concatenate([_layernorm(h) for h in hs], axis=0)
            h = jnp.concatenate(hs, axis=0)
            FH = F // 2

            lh = _strassen_lhs(hn[:HX, 0:256], hn[:HX, 256:512], hn[HX:, 0:256], hn[HX:, 256:512])
            hr = hn[:, 512:D].astype(bf16)

            def proj(w, c):
                a, b = slice(c, c + 128), slice(FH + c, FH + c + 128)
                left, right = _strassen(lh, w[0:256, a], w[0:256, b], w[256:512, a], w[256:512, b])
                return left + _dot(hr, w[512:D, a]), right + _dot(hr, w[512:D, b])

            al, ar = [], []
            for c in range(0, FH, 128):
                (gl, gr), (ul, ur) = proj(wg_v, c), proj(wu_v, c)
                al.append(_gelu(gl) * ul)
                ar.append(_gelu(gr) * ur)
            act = jnp.concatenate(al + ar, axis=1)

            la = _strassen_lhs(act[:HX, :FH], act[:HX, FH:], act[HX:, :FH], act[HX:, FH:])
            for c in range(0, 256, 128):
                a, b = slice(c, c + 128), slice(256 + c, 256 + c + 128)
                left, right = _strassen(la, wd_v[0:FH, a], wd_v[0:FH, b], wd_v[FH:F, a], wd_v[FH:F, b])
                out_v[pl.ds(row, TS), a] = (h[:, a] + left).astype(bf16)
                out_v[pl.ds(row, TS), b] = (h[:, b] + right).astype(bf16)
            out_copy(t, 0).start()
            for k, r0 in enumerate((0, HX)):
                y = _dot(act[r0:r0 + HX].astype(bf16), wd_v[:, 512:D])
                out_v[pl.ds(pl.multiple_of(row + r0, 128), HX), 512:D] = (h[r0:r0 + HX, 512:D] + y).astype(bf16)
                out_copy(t, 1 + k).start()
            return carry

        lax.fori_loop(0, n, p2, 0)
        for t in range(n):
            for c in range(NOC):
                out_copy(t, c).wait()


_SCRATCH = [
    pltpu.VMEM((S, D), bf16),
    pltpu.VMEM((D, 3 * D), bf16),
    pltpu.VMEM((DH, DH, H), bf16),
    pltpu.VMEM((D, D), bf16),
    pltpu.VMEM((D, F), bf16),
    pltpu.VMEM((D, F), bf16),
    pltpu.VMEM((F, D), bf16),
    pltpu.VMEM((S, D), bf16),
    pltpu.VMEM((NL, D), bf16),
    pltpu.VMEM((D, D), bf16),
    pltpu.VMEM((NL, D), bf16),
    pltpu.VMEM((D, D), bf16),
    pltpu.VMEM((2, TS, D), bf16),
    pltpu.VMEM((KV_OFF[-1], 128), bf16),
    pltpu.VMEM((KV_OFF[-1], 128), f32),
    pltpu.VMEM((FOLD_OFF[-1], 128), bf16),
    pltpu.VMEM((2, KV_OFF[-1], TS), bf16),
    pltpu.VMEM((NTILE, NFT * 128, TS), bf16),
    pltpu.SemaphoreType.DMA((10 + NTILE,)),
    pltpu.SemaphoreType.DMA((NTILE * NOC,)),
]


def _compiler_params():
    kw = dict(dimension_semantics=("arbitrary",), vmem_limit_bytes=100 * 1024 * 1024,
              disable_bounds_checks=True, disable_semaphore_checks=True)
    known = {f.name for f in dataclasses.fields(pltpu.CompilerParams)}
    return pltpu.CompilerParams(**{k: v for k, v in kw.items() if k in known})


@jax.jit
def pallas_sequential_preLN__linear_kernel_hedgehog__geglu_ffn__prompt_kernel(
    A_x: jax.Array,
    A_wqkv: jax.Array,
    A_w_phi: jax.Array,
    A_wo: jax.Array,
    B_x: jax.Array,
    B_w_gate: jax.Array,
    B_w_up: jax.Array,
    B_w_down: jax.Array,
):
    del B_x
    return pl.pallas_call(
        _kernel,
        out_shape=jax.ShapeDtypeStruct(A_x.shape, A_x.dtype),
        grid=(2,),
        in_specs=[pl.BlockSpec(memory_space=pl.ANY)] * 7,
        out_specs=pl.BlockSpec(memory_space=pl.ANY),
        scratch_shapes=_SCRATCH,
        compiler_params=_compiler_params(),
    )(A_x, A_wqkv, jnp.transpose(A_w_phi, (1, 2, 0)), A_wo, B_w_gate, B_w_up, B_w_down)
```

```python
import dataclasses

import jax
import jax.numpy as jnp
from jax import lax
import jax.experimental.pallas as pl
import jax.experimental.pallas.tpu as pltpu

S, D, H, DH, F = 2048, 640, 32, 20, 1536
NG = H // 2
EPS = 1e-5
DEN_EPS = 1e-6
LOG2E = 1.4426950408889634
NT = (((1,), (1,)), ((), ()))
f32, bf16 = jnp.float32, jnp.bfloat16

TS = 512
NTILE = S // TS
HX = TS // 2
VA = 256
A0, A1, B1 = 320, 512, 512
VS = 480
NA = 4
WR = 64
OCH = ((0, TS, 0, 256), (0, TS, 256, 512), (0, 448, 512, D), (448, TS, 512, D))
NOC = len(OCH)

NFT = 11
KV_W = [(60 * i - 4 * (i % 2), 60 * i - 4 * (i % 2) + 64) for i in range(NFT - 1)] + [(600, 640)]
KV_J = [0 if i % 2 else 60 for i in range(NFT - 1)] + [40]
KV_L = [64] * (NFT - 1) + [48]
KV_OFF = [sum(KV_L[:i]) for i in range(NFT + 1)]

NM, NL = 16 * H, 19 * H
FOLD_H = [(128 * t // DH, (128 * t + 127) // DH) for t in range(5)]
FOLD_M = [(16 * h0, 16 * h1 + 16) for h0, h1 in FOLD_H]
FOLD_T = [(32 * (h0 // 8), 32 * (h1 // 8) + 32) for h0, h1 in FOLD_H]
FOLD_OFF = [sum(m1 - m0 + t1 - t0 for (m0, m1), (t0, t1) in zip(FOLD_M[:i], FOLD_T[:i]))
            for i in range(6)]


def _iota(shape, dim):
    return lax.broadcasted_iota(jnp.int32, shape, dim)


def _dot(a, b):
    return jnp.dot(a, b, preferred_element_type=f32)


def _dot_nt(a, b):
    return lax.dot_general(a, b, NT, preferred_element_type=f32)


def _assemble(parts, ranges, total):
    cuts = sorted({0, total} | {r for rr in ranges for r in rr})
    segs = []
    for a, b in zip(cuts[:-1], cuts[1:]):
        acc = None
        for p, (r0, r1) in zip(parts, ranges):
            if r0 <= a and b <= r1:
                piece = p[a - r0:b - r0]
                acc = piece if acc is None else acc + piece
        segs.append(acc)
    return jnp.concatenate(segs, axis=0)


def _layernorm(x):
    m = jnp.sum(x, axis=-1, keepdims=True) * (1.0 / D)
    xc = x - m
    v = jnp.sum(xc * xc, axis=-1, keepdims=True) * (1.0 / D)
    return xc * lax.rsqrt(v + EPS)


def _gelu(x):
    c = 0.7978845608028654
    return 0.5 * x * (1.0 + jnp.tanh(c * (x + 0.044715 * (x * x * x))))


def _strassen_lhs(a11, a12, a21, a22):
    return [x.astype(bf16) for x in (a11 + a22, a21 + a22, a11, a22, a11 + a12, a21 - a11, a12 - a22)]


def _strassen(la, b11, b12, b21, b22):
    f11, f12, f21, f22 = (b.astype(f32) for b in (b11, b12, b21, b22))
    m3 = _dot(la[2], (f12 - f22).astype(bf16))
    m5 = _dot(la[4], b22)
    c12 = m3 + m5
    m1 = _dot(la[0], (f11 + f22).astype(bf16))
    c11, c22 = m1 - m5, m1 + m3
    m4 = _dot(la[3], (f21 - f11).astype(bf16))
    c11 = c11 + m4
    c11 = c11 + _dot(la[6], (f21 + f22).astype(bf16))
    m2 = _dot(la[1], b11)
    c21, c22 = m2 + m4, c22 - m2
    c22 = c22 + _dot(la[5], (f11 + f12).astype(bf16))
    return jnp.concatenate([c11, c21], axis=0), jnp.concatenate([c12, c22], axis=0)


def _feat(pT, scaled=False):
    ts = pT.shape[1]
    p = pT.reshape(4, 19, 8, ts)
    sub = _iota((4, 8, ts), 1)
    es = [p[:, 0], p[:, 1], p[:, 2], jnp.zeros((4, 8, ts), f32)]
    for d in (1, 2):
        lo = (sub & (2 * d)) == 0
        for i in (0, 2 if d == 1 else 1):
            x, y = es[i], es[i + d]
            es[i] = jnp.where(lo, x, pltpu.roll(y, 2 * d, 1))
            es[i + d] = jnp.where(lo, pltpu.roll(x, 8 - 2 * d, 1), y)
    p = jnp.stack([v for i in range(4) for v in (
        p[:, 3 + 4 * i], p[:, 4 + 4 * i], es[i], p[:, 5 + 4 * i], p[:, 6 + 4 * i])], axis=1)
    p = p.reshape(NG, 5, 8, ts)
    even = _iota((NG, 8, ts), 1) % 2 == 0

    def red(op, x):
        a, b = op(x[:, 0], x[:, 1]), op(x[:, 3], x[:, 4])
        c = op(jnp.where(even, a, b), pltpu.roll(jnp.where(even, b, a), 1, 1))
        c = op(c, x[:, 2])
        c = op(c, pltpu.roll(c, 2, 1))
        return op(c, pltpu.roll(c, 4, 1))

    def spread(c):
        ca, cb = jnp.broadcast_to(c[:, 0:1], c.shape), jnp.broadcast_to(c[:, 1:2], c.shape)
        return jnp.stack([ca, ca, c, cb, cb], axis=1)

    ep = jnp.exp2(p - spread(red(jnp.maximum, p)))
    en = jnp.exp2(spread(red(jnp.minimum, p)) - p)
    sp, rn = red(jnp.add, ep), pl.reciprocal(red(jnp.add, en), approx=True)
    if scaled:
        en = en * spread(rn * sp)
    else:
        ep = ep * spread(pl.reciprocal(sp, approx=True))
        en = en * spread(rn)
    ma = jnp.where(even, ep[:, 2], pltpu.roll(en[:, 2], 1, 1))
    mb = jnp.where(even, pltpu.roll(ep[:, 2], 1, 1), en[:, 2])
    phi = jnp.concatenate([ep[:, 0:2], en[:, 0:2], ma[:, None],
                           ep[:, 3:5], en[:, 3:5], mb[:, None]], axis=1).reshape(2 * D, ts)
    tiles = []
    for i in range(NFT):
        w = phi[120 * i:120 * i + 120]
        tiles.append(jnp.concatenate([w, jnp.zeros((128 - w.shape[0], ts), f32)], axis=0))
    return tiles


def _kernel(x_hbm, wqkv_hbm, wphi_hbm, wo_hbm, wg_hbm, wu_hbm, wd_hbm, o_hbm,
            x_v, wqkv_v, wphi_v, wo_v, wg_v, wu_v, wd_v, out_v,
            wkT, wvT, wqT, perm_s, xn_s, kvT, kv_acc, bdt_s, lhs_s, fq_s, sems, osems):
    n = NTILE

    @pl.when(pl.program_id(0) == 0)
    def _phase1():
        def wblock(r0, nr, c0, s):
            return pltpu.make_async_copy(wqkv_hbm.at[pl.ds(r0, nr), pl.ds(c0, D)],
                                         wqkv_v.at[pl.ds(r0, nr), pl.ds(c0, D)], sems.at[s])

        def xrows(row, nr, s):
            return pltpu.make_async_copy(x_hbm.at[0, pl.ds(row, nr)], x_v.at[pl.ds(row, nr)], sems.at[s])

        def cp_x(t):
            return xrows(pl.multiple_of(t * TS, TS), TS, 10 + t)

        cp_phi = pltpu.make_async_copy(wphi_hbm, wphi_v, sems.at[0])
        cp_x0a, cp_x0b = xrows(0, HX, 9), xrows(HX, HX, 10)
        cp_va, cp_vb = wblock(0, VA, 2 * D, 1), wblock(VA, D - VA, 2 * D, 2)
        cp_k, cp_q = wblock(0, D, D, 3), wblock(0, D, 0, 4)
        cp_ffn = [pltpu.make_async_copy(src, dst, sems.at[5 + j]) for j, (src, dst) in enumerate(
            [(wo_hbm, wo_v), (wg_hbm, wg_v), (wu_hbm, wu_v), (wd_hbm, wd_v)])]
        for c in ([cp_phi, cp_x0a, cp_va, cp_x0b, cp_vb, cp_k, cp_q]
                  + [cp_x(t) for t in range(1, n)] + cp_ffn):
            c.start()

        def put_lhs(t, vT, base=0):
            lo = _iota((8, TS), 0) < 4
            for i, (r0, r1) in enumerate(KV_W):
                if r0 < base or r1 > base + vT.shape[0]:
                    continue
                w = vT[r0 - base:r1 - base]
                if i == NFT - 1:
                    w = jnp.concatenate([w, jnp.ones((8, TS), f32)], axis=0)
                elif i % 2:
                    w = jnp.concatenate([jnp.where(lo, 1.0, w[0:8]), w[8:]], axis=0)
                else:
                    w = jnp.concatenate([w[:56], jnp.where(lo, w[56:64], 1.0)], axis=0)
                lhs_s[t % 2, KV_OFF[i]:KV_OFF[i + 1], :] = w.astype(bf16)

        def put_feat(slot, phi):
            for i in range(NFT):
                fq_s[slot, 128 * i:128 * i + 128, :] = phi[i].astype(bf16)

        def put_kv(kv):
            for i in range(NFT):
                kv_acc[KV_OFF[i]:KV_OFF[i + 1], :] = kv[i]

        def PK(t):
            return _feat(_dot_nt(wkT[...], xn_s[t % 2]))

        def PQ(t):
            put_feat(t, _feat(_dot_nt(wqT[...], xn_s[t % 2]), scaled=True))

        def LNPV(t):
            row = pl.multiple_of(t * TS, TS)
            xn = _layernorm(x_v[pl.ds(row, TS), :].astype(f32)).astype(bf16)
            xn_s[t % 2] = xn
            put_lhs(t, _dot_nt(wvT[0:VS, :], xn))

        def PVB(t):
            put_lhs(t, _dot_nt(wvT[VS:D, :], xn_s[t % 2]), VS)

        def KV(t, phi):
            return [kv_acc[KV_OFF[i]:KV_OFF[i + 1], :]
                    + _dot_nt(lhs_s[t % 2, KV_OFF[i]:KV_OFF[i + 1], :], phi[i].astype(bf16))
                    for i in range(NFT)]

        def fold(off):
            parts = [_dot_nt(bdt_s[FOLD_OFF[t]:FOLD_OFF[t + 1], :],
                             wqkv_v[:, off + 128 * t:off + 128 * t + 128]) for t in range(5)]
            nm = [m1 - m0 for m0, m1 in FOLD_M]
            wm = _assemble([p[:k] for p, k in zip(parts, nm)], FOLD_M, NM)
            wt = _assemble([p[k:] for p, k in zip(parts, nm)], FOLD_T, 4 * H).reshape(4, 4, 8, D)
            ref = wt[:, 3]
            refm = jnp.concatenate([jnp.broadcast_to(ref[h // 8, h % 8:h % 8 + 1], (16, D))
                                    for h in range(H)], axis=0)
            w = jnp.concatenate([wt[:, :3] - ref[:, None], (wm - refm).reshape(4, 16, 8, D)], axis=1)
            return (w.reshape(NL, D) * LOG2E).astype(bf16)

        kk = _iota((D, 1), 0)
        perm_s[...] = jnp.where(_iota((1, D), 1) == DH * (kk % H) + kk // H, 1.0, 0.0).astype(bf16)
        cp_phi.wait()
        q = jnp.concatenate([wphi_v[d].astype(f32) for d in range(DH)], axis=1).astype(bf16)
        tf = _dot(q, perm_s[...])
        hc = _iota((1, D), 1) // DH
        for t, (h0, h1) in enumerate(FOLD_H):
            tt, ht = tf[:, 128 * t:128 * t + 128], hc[:, 128 * t:128 * t + 128]
            blk = [jnp.where(ht == h, tt[:16], 0.0) for h in range(h0, h1 + 1)]
            for g in range(h0 // 8, h1 // 8 + 1):
                keep = _iota((8, 1), 0) + 8 * g == ht
                blk += [jnp.where(keep, jnp.broadcast_to(tt[16 + k:17 + k], (8, 128)), 0.0)
                        for k in range(4)]
            bdt_s[FOLD_OFF[t]:FOLD_OFF[t + 1], :] = jnp.concatenate(blk, axis=0).astype(bf16)

        def pva(r0, r1, s0, s1):
            return _dot_nt(wvT[r0:r1, 0:VA], xn_s[0, s0:s1, 0:VA])

        def pvb(r0, r1):
            return _dot_nt(wvT[r0:r1, VA:D], xn_s[0, :, VA:D])

        cp_x0a.wait()
        xn_s[0, 0:HX, :] = _layernorm(x_v[0:HX, :].astype(f32)).astype(bf16)
        cp_va.wait()
        wvT[:, 0:VA] = wqkv_v[0:VA, 2 * D:3 * D].T
        paa = pva(0, A0, 0, HX)
        cp_x0b.wait()
        paa = jnp.concatenate([paa, pva(A0, D, 0, HX)], axis=0)
        xn_s[0, HX:TS, :] = _layernorm(x_v[HX:TS, :].astype(f32)).astype(bf16)
        pab = pva(0, A1, HX, TS)
        cp_vb.wait()
        pab = jnp.concatenate([pab, pva(A1, D, HX, TS)], axis=0)
        pa = jnp.concatenate([paa, pab], axis=1)
        wvT[:, VA:D] = wqkv_v[VA:D, 2 * D:3 * D].T
        v0 = pa[0:B1] + pvb(0, B1)
        cp_k.wait()
        wkT[...] = fold(D)
        put_feat(n - 1, PK(0))
        put_lhs(0, jnp.concatenate([v0, pa[B1:D] + pvb(B1, D)], axis=0))
        cp_q.wait()
        cp_x(1).wait()
        wqT[...] = fold(0)
        PQ(0)
        put_kv([_dot_nt(lhs_s[0, KV_OFF[i]:KV_OFF[i + 1], :], fq_s[n - 1, 128 * i:128 * i + 128, :])
                for i in range(NFT)])
        LNPV(1)

        def p1(t, carry):
            cp_x(t + 1).wait()
            fk = PK(t)
            PQ(t)
            PVB(t)
            kv = KV(t, fk)
            LNPV(t + 1)
            put_kv(kv)
            return carry
        lax.fori_loop(1, n - 1, p1, 0)

        fk = PK(n - 1)
        PQ(n - 1)
        PVB(n - 1)
        kv = KV(n - 1, fk)
        cc = _iota((1, 128), 1)
        plus_c = jnp.logical_or(cc % 40 < 16, jnp.logical_and(cc % 40 >= 32, cc % 2 == 0))
        eps_c = jnp.where(plus_c, DEN_EPS, 0.0)
        for i, (r0, r1) in enumerate(KV_W):
            j_c = jnp.where(cc < min(120, 2 * D - 120 * i), cc // 40, -64)
            rr = _iota((KV_L[i], 1), 0)
            dlt = rr - (DH * j_c + (60 * i - r0))
            zrow = rr - KV_J[i] == j_c
            keep = jnp.logical_or(jnp.logical_and(dlt >= 0, dlt < DH), zrow)
            kvT[KV_OFF[i]:KV_OFF[i + 1], :] = (jnp.where(keep, kv[i], 0.0)
                                               + jnp.where(zrow, eps_c, 0.0)).astype(bf16)
        for c in cp_ffn:
            c.wait()

    @pl.when(pl.program_id(0) == 1)
    def _phase2():
        def out_copy(t, c):
            r0, r1, c0, c1 = OCH[c]
            row = pl.multiple_of(t * TS + r0, 64)
            return pltpu.make_async_copy(out_v.at[pl.ds(row, r1 - r0), pl.ds(c0, c1 - c0)],
                                         o_hbm.at[0, pl.ds(row, r1 - r0), pl.ds(c0, c1 - c0)],
                                         osems.at[t * NOC + c])

        def attn_o(t, c0, c1):
            m = c1 - c0
            parts = [_dot(kvT[KV_OFF[i]:KV_OFF[i + 1], :], fq_s[t, 128 * i:128 * i + 128, c0:c1])
                     for i in range(NFT)]
            sub = _iota((8, m), 0)
            lo = sub < 4
            segs, rds = [], []
            for i in range(0, NFT - 1, 2):
                pe, po = parts[i], parts[i + 1]
                segs += [pe[:56], jnp.where(lo, pe[56:64], po[0:8]), po[8:]]
                rd = 1.0 / jnp.where(sub % 4 == 3, 1.0, jnp.where(lo, po[0:8], pe[56:64]))
                rds += [rd[j:j + 1] for j in (4, 5, 6, 0, 1, 2)]
            segs.append(parts[NFT - 1][:40])
            rd = 1.0 / jnp.where(sub < 2, parts[NFT - 1][40:48], 1.0)
            rds += [rd[0:1], rd[1:2]]
            scale = []
            for g in range(NG):
                a0 = jnp.broadcast_to(rds[2 * g], (8, m))
                a1 = jnp.broadcast_to(rds[2 * g + 1], (8, m))
                scale += [a0, a0, jnp.where(lo, a0, a1), a1, a1]
            return (jnp.concatenate(segs, axis=0) * jnp.concatenate(scale, axis=0)).T

        def p2(t, carry):
            row = pl.multiple_of(t * TS, TS)
            ma = TS // NA
            o = jnp.concatenate([attn_o(t, j * ma, (j + 1) * ma) for j in range(NA)], axis=0)
            hs = [x_v[pl.ds(row + r0, WR), :].astype(f32) + _dot(o[r0:r0 + WR].astype(bf16), wo_v[...])
                  for r0 in range(0, TS, WR)]
            hn = jnp.concatenate([_layernorm(h) for h in hs], axis=0)
            h = jnp.concatenate(hs, axis=0)
            FH = F // 2

            lh = _strassen_lhs(hn[:HX, 0:256], hn[:HX, 256:512], hn[HX:, 0:256], hn[HX:, 256:512])
            hr = hn[:, 512:D].astype(bf16)

            def proj(w, c):
                a, b = slice(c, c + 128), slice(FH + c, FH + c + 128)
                left, right = _strassen(lh, w[0:256, a], w[0:256, b], w[256:512, a], w[256:512, b])
                return left + _dot(hr, w[512:D, a]), right + _dot(hr, w[512:D, b])

            al, ar = [], []
            for c in range(0, FH, 128):
                (gl, gr), (ul, ur) = proj(wg_v, c), proj(wu_v, c)
                al.append(_gelu(gl) * ul)
                ar.append(_gelu(gr) * ur)
            act = jnp.concatenate(al + ar, axis=1)

            la = _strassen_lhs(act[:HX, :FH], act[:HX, FH:], act[HX:, :FH], act[HX:, FH:])
            for k, c in enumerate((0, 256)):
                a, b = slice(c, c + 128), slice(c + 128, c + 256)
                left, right = _strassen(la, wd_v[0:FH, a], wd_v[0:FH, b], wd_v[FH:F, a], wd_v[FH:F, b])
                out_v[pl.ds(row, TS), c:c + 256] = (
                    h[:, c:c + 256] + jnp.concatenate([left, right], axis=1)).astype(bf16)
                out_copy(t, k).start()
            for k, (r0, r1, _, _) in enumerate(OCH[2:]):
                y = _dot(act[r0:r1].astype(bf16), wd_v[:, 512:D])
                out_v[pl.ds(pl.multiple_of(row + r0, 64), r1 - r0), 512:D] = (h[r0:r1, 512:D] + y).astype(bf16)
                out_copy(t, 2 + k).start()
            return carry

        lax.fori_loop(0, n, p2, 0)
        for t in range(n):
            for c in range(NOC):
                out_copy(t, c).wait()


_SCRATCH = [
    pltpu.VMEM((S, D), bf16),
    pltpu.VMEM((D, 3 * D), bf16),
    pltpu.VMEM((DH, DH, H), bf16),
    pltpu.VMEM((D, D), bf16),
    pltpu.VMEM((D, F), bf16),
    pltpu.VMEM((D, F), bf16),
    pltpu.VMEM((F, D), bf16),
    pltpu.VMEM((S, D), bf16),
    pltpu.VMEM((NL, D), bf16),
    pltpu.VMEM((D, D), bf16),
    pltpu.VMEM((NL, D), bf16),
    pltpu.VMEM((D, D), bf16),
    pltpu.VMEM((2, TS, D), bf16),
    pltpu.VMEM((KV_OFF[-1], 128), bf16),
    pltpu.VMEM((KV_OFF[-1], 128), f32),
    pltpu.VMEM((FOLD_OFF[-1], 128), bf16),
    pltpu.VMEM((2, KV_OFF[-1], TS), bf16),
    pltpu.VMEM((NTILE, NFT * 128, TS), bf16),
    pltpu.SemaphoreType.DMA((10 + NTILE,)),
    pltpu.SemaphoreType.DMA((NTILE * NOC,)),
]


def _compiler_params():
    kw = dict(dimension_semantics=("arbitrary",), vmem_limit_bytes=100 * 1024 * 1024,
              disable_bounds_checks=True, disable_semaphore_checks=True)
    known = {f.name for f in dataclasses.fields(pltpu.CompilerParams)}
    return pltpu.CompilerParams(**{k: v for k, v in kw.items() if k in known})


@jax.jit
def pallas_sequential_preLN__linear_kernel_hedgehog__geglu_ffn__prompt_kernel(
    A_x: jax.Array,
    A_wqkv: jax.Array,
    A_w_phi: jax.Array,
    A_wo: jax.Array,
    B_x: jax.Array,
    B_w_gate: jax.Array,
    B_w_up: jax.Array,
    B_w_down: jax.Array,
):
    del B_x
    return pl.pallas_call(
        _kernel,
        out_shape=jax.ShapeDtypeStruct(A_x.shape, A_x.dtype),
        grid=(2,),
        in_specs=[pl.BlockSpec(memory_space=pl.ANY)] * 7,
        out_specs=pl.BlockSpec(memory_space=pl.ANY),
        scratch_shapes=_SCRATCH,
        compiler_params=_compiler_params(),
    )(A_x, A_wqkv, jnp.transpose(A_w_phi, (1, 2, 0)), A_wo, B_w_gate, B_w_up, B_w_down)
```

```python
import dataclasses

import jax
import jax.numpy as jnp
from jax import lax
import jax.experimental.pallas as pl
import jax.experimental.pallas.tpu as pltpu

S, D, H, DH, F = 2048, 640, 32, 20, 1536
NG = H // 2
EPS = 1e-5
DEN_EPS = 1e-6
LOG2E = 1.4426950408889634
NT = (((1,), (1,)), ((), ()))
f32, bf16 = jnp.float32, jnp.bfloat16

TS = 512
NTILE = S // TS
HX = TS // 2
VA = 256
A0, A1, B1 = 320, 512, 512
VS = 480
NA = 4
WR = 64
OCH = ((0, TS, 0, 256), (0, TS, 256, 512), (0, 448, 512, D), (448, TS, 512, D))
NOC = len(OCH)

NFT = 11
KV_W = [(60 * i - 4 * (i % 2), 60 * i - 4 * (i % 2) + 64) for i in range(NFT - 1)] + [(600, 640)]
KV_J = [0 if i % 2 else 60 for i in range(NFT - 1)] + [40]
KV_L = [64] * (NFT - 1) + [48]
KV_OFF = [sum(KV_L[:i]) for i in range(NFT + 1)]

NM, NL = 16 * H, 19 * H
FOLD_H = [(128 * t // DH, (128 * t + 127) // DH) for t in range(5)]
FOLD_M = [(16 * h0, 16 * h1 + 16) for h0, h1 in FOLD_H]
FOLD_T = [(32 * (h0 // 8), 32 * (h1 // 8) + 32) for h0, h1 in FOLD_H]
FOLD_OFF = [sum(m1 - m0 + t1 - t0 for (m0, m1), (t0, t1) in zip(FOLD_M[:i], FOLD_T[:i]))
            for i in range(6)]


def _iota(shape, dim):
    return lax.broadcasted_iota(jnp.int32, shape, dim)


def _dot(a, b):
    return jnp.dot(a, b, preferred_element_type=f32)


def _dot_nt(a, b):
    return lax.dot_general(a, b, NT, preferred_element_type=f32)


def _assemble(parts, ranges, total):
    cuts = sorted({0, total} | {r for rr in ranges for r in rr})
    segs = []
    for a, b in zip(cuts[:-1], cuts[1:]):
        acc = None
        for p, (r0, r1) in zip(parts, ranges):
            if r0 <= a and b <= r1:
                piece = p[a - r0:b - r0]
                acc = piece if acc is None else acc + piece
        segs.append(acc)
    return jnp.concatenate(segs, axis=0)


def _layernorm(x):
    m = jnp.sum(x, axis=-1, keepdims=True) * (1.0 / D)
    xc = x - m
    v = jnp.sum(xc * xc, axis=-1, keepdims=True) * (1.0 / D)
    return xc * lax.rsqrt(v + EPS)


def _gelu(x):
    c = 0.7978845608028654
    return 0.5 * x * (1.0 + jnp.tanh(c * (x + 0.044715 * (x * x * x))))


def _strassen_lhs(a11, a12, a21, a22):
    return [x.astype(bf16) for x in (a11 + a22, a21 + a22, a11, a22, a11 + a12, a21 - a11, a12 - a22)]


def _strassen(la, b11, b12, b21, b22):
    f11, f12, f21, f22 = (b.astype(f32) for b in (b11, b12, b21, b22))
    m3 = _dot(la[2], (f12 - f22).astype(bf16))
    m5 = _dot(la[4], b22)
    c12 = m3 + m5
    m1 = _dot(la[0], (f11 + f22).astype(bf16))
    c11, c22 = m1 - m5, m1 + m3
    m4 = _dot(la[3], (f21 - f11).astype(bf16))
    c11 = c11 + m4
    c11 = c11 + _dot(la[6], (f21 + f22).astype(bf16))
    m2 = _dot(la[1], b11)
    c21, c22 = m2 + m4, c22 - m2
    c22 = c22 + _dot(la[5], (f11 + f12).astype(bf16))
    return jnp.concatenate([c11, c21], axis=0), jnp.concatenate([c12, c22], axis=0)


def _feat(pT, scaled=False):
    ts = pT.shape[1]
    p = pT.reshape(4, 19, 8, ts)
    sub = _iota((4, 8, ts), 1)
    es = [p[:, 0], p[:, 1], p[:, 2], jnp.zeros((4, 8, ts), f32)]
    for d in (1, 2):
        lo = (sub & (2 * d)) == 0
        for i in (0, 2 if d == 1 else 1):
            x, y = es[i], es[i + d]
            es[i] = jnp.where(lo, x, pltpu.roll(y, 2 * d, 1))
            es[i + d] = jnp.where(lo, pltpu.roll(x, 8 - 2 * d, 1), y)
    p = jnp.stack([v for i in range(4) for v in (
        p[:, 3 + 4 * i], p[:, 4 + 4 * i], es[i], p[:, 5 + 4 * i], p[:, 6 + 4 * i])], axis=1)
    p = p.reshape(NG, 5, 8, ts)
    even = _iota((NG, 8, ts), 1) % 2 == 0

    def red(op, x):
        a, b = op(x[:, 0], x[:, 1]), op(x[:, 3], x[:, 4])
        c = op(jnp.where(even, a, b), pltpu.roll(jnp.where(even, b, a), 1, 1))
        c = op(c, x[:, 2])
        c = op(c, pltpu.roll(c, 2, 1))
        return op(c, pltpu.roll(c, 4, 1))

    def spread(c):
        ca, cb = jnp.broadcast_to(c[:, 0:1], c.shape), jnp.broadcast_to(c[:, 1:2], c.shape)
        return jnp.stack([ca, ca, c, cb, cb], axis=1)

    ep = jnp.exp2(p - spread(red(jnp.maximum, p)))
    en = jnp.exp2(spread(red(jnp.minimum, p)) - p)
    sp, rn = red(jnp.add, ep), pl.reciprocal(red(jnp.add, en), approx=True)
    if scaled:
        en = en * spread(rn * sp)
    else:
        ep = ep * spread(pl.reciprocal(sp, approx=True))
        en = en * spread(rn)
    ma = jnp.where(even, ep[:, 2], pltpu.roll(en[:, 2], 1, 1))
    mb = jnp.where(even, pltpu.roll(ep[:, 2], 1, 1), en[:, 2])
    phi = jnp.concatenate([ep[:, 0:2], en[:, 0:2], ma[:, None],
                           ep[:, 3:5], en[:, 3:5], mb[:, None]], axis=1).reshape(2 * D, ts)
    tiles = []
    for i in range(NFT):
        w = phi[120 * i:120 * i + 120]
        tiles.append(jnp.concatenate([w, jnp.zeros((128 - w.shape[0], ts), f32)], axis=0))
    return tiles


def _kernel(x_hbm, wqkv_hbm, wphi_hbm, wo_hbm, wg_hbm, wu_hbm, wd_hbm, o_hbm,
            x_v, wqkv_v, wphi_v, wo_v, wg_v, wu_v, wd_v, out_v,
            wkT, wvT, wqT, perm_s, xn_s, kvT, kv_acc, bdt_s, lhs_s, fq_s, sems, osems):
    n = NTILE

    @pl.when(pl.program_id(0) == 0)
    def _phase1():
        def wblock(r0, nr, c0, s):
            return pltpu.make_async_copy(wqkv_hbm.at[pl.ds(r0, nr), pl.ds(c0, D)],
                                         wqkv_v.at[pl.ds(r0, nr), pl.ds(c0, D)], sems.at[s])

        def xrows(row, nr, s):
            return pltpu.make_async_copy(x_hbm.at[0, pl.ds(row, nr)], x_v.at[pl.ds(row, nr)], sems.at[s])

        def cp_x(t):
            return xrows(pl.multiple_of(t * TS, TS), TS, 10 + t)

        cp_phi = pltpu.make_async_copy(wphi_hbm, wphi_v, sems.at[0])
        cp_x0a, cp_x0b = xrows(0, HX, 9), xrows(HX, HX, 10)
        cp_va, cp_vb = wblock(0, VA, 2 * D, 1), wblock(VA, D - VA, 2 * D, 2)
        cp_k, cp_q = wblock(0, D, D, 3), wblock(0, D, 0, 4)
        cp_ffn = [pltpu.make_async_copy(src, dst, sems.at[5 + j]) for j, (src, dst) in enumerate(
            [(wo_hbm, wo_v), (wg_hbm, wg_v), (wu_hbm, wu_v), (wd_hbm, wd_v)])]
        for c in ([cp_phi, cp_x0a, cp_va, cp_x0b, cp_vb, cp_k, cp_q]
                  + [cp_x(t) for t in range(1, n)] + cp_ffn):
            c.start()

        def put_lhs(t, vT, base=0):
            lo = _iota((8, TS), 0) < 4
            for i, (r0, r1) in enumerate(KV_W):
                if r0 < base or r1 > base + vT.shape[0]:
                    continue
                w = vT[r0 - base:r1 - base]
                if i == NFT - 1:
                    w = jnp.concatenate([w, jnp.ones((8, TS), f32)], axis=0)
                elif i % 2:
                    w = jnp.concatenate([jnp.where(lo, 1.0, w[0:8]), w[8:]], axis=0)
                else:
                    w = jnp.concatenate([w[:56], jnp.where(lo, w[56:64], 1.0)], axis=0)
                lhs_s[t % 2, KV_OFF[i]:KV_OFF[i + 1], :] = w.astype(bf16)

        def put_feat(slot, phi):
            for i in range(NFT):
                fq_s[slot, 128 * i:128 * i + 128, :] = phi[i].astype(bf16)

        def put_kv(kv):
            for i in range(NFT):
                kv_acc[KV_OFF[i]:KV_OFF[i + 1], :] = kv[i]

        def PK(t):
            return _feat(_dot_nt(wkT[...], xn_s[t % 2]))

        def PQ(t):
            put_feat(t, _feat(_dot_nt(wqT[...], xn_s[t % 2]), scaled=True))

        def LNPV(t):
            row = pl.multiple_of(t * TS, TS)
            xn = _layernorm(x_v[pl.ds(row, TS), :].astype(f32)).astype(bf16)
            xn_s[t % 2] = xn
            put_lhs(t, _dot_nt(wvT[0:VS, :], xn))

        def PVB(t):
            put_lhs(t, _dot_nt(wvT[VS:D, :], xn_s[t % 2]), VS)

        def KV(t, phi):
            return [kv_acc[KV_OFF[i]:KV_OFF[i + 1], :]
                    + _dot_nt(lhs_s[t % 2, KV_OFF[i]:KV_OFF[i + 1], :], phi[i].astype(bf16))
                    for i in range(NFT)]

        def fold(off):
            parts = [_dot_nt(bdt_s[FOLD_OFF[t]:FOLD_OFF[t + 1], :],
                             wqkv_v[:, off + 128 * t:off + 128 * t + 128]) for t in range(5)]
            nm = [m1 - m0 for m0, m1 in FOLD_M]
            wm = _assemble([p[:k] for p, k in zip(parts, nm)], FOLD_M, NM)
            wt = _assemble([p[k:] for p, k in zip(parts, nm)], FOLD_T, 4 * H).reshape(4, 4, 8, D)
            ref = wt[:, 3]
            refm = jnp.concatenate([jnp.broadcast_to(ref[h // 8, h % 8:h % 8 + 1], (16, D))
                                    for h in range(H)], axis=0)
            w = jnp.concatenate([wt[:, :3] - ref[:, None], (wm - refm).reshape(4, 16, 8, D)], axis=1)
            return (w.reshape(NL, D) * LOG2E).astype(bf16)

        kk = _iota((D, 1), 0)
        perm_s[...] = jnp.where(_iota((1, D), 1) == DH * (kk % H) + kk // H, 1.0, 0.0).astype(bf16)
        cp_phi.wait()
        q = jnp.concatenate([wphi_v[d].astype(f32) for d in range(DH)], axis=1).astype(bf16)
        tf = _dot(q, perm_s[...])
        hc = _iota((1, D), 1) // DH
        for t, (h0, h1) in enumerate(FOLD_H):
            tt, ht = tf[:, 128 * t:128 * t + 128], hc[:, 128 * t:128 * t + 128]
            blk = [jnp.where(ht == h, tt[:16], 0.0) for h in range(h0, h1 + 1)]
            for g in range(h0 // 8, h1 // 8 + 1):
                keep = _iota((8, 1), 0) + 8 * g == ht
                blk += [jnp.where(keep, jnp.broadcast_to(tt[16 + k:17 + k], (8, 128)), 0.0)
                        for k in range(4)]
            bdt_s[FOLD_OFF[t]:FOLD_OFF[t + 1], :] = jnp.concatenate(blk, axis=0).astype(bf16)

        def pva(r0, r1, s0, s1):
            return _dot_nt(wvT[r0:r1, 0:VA], xn_s[0, s0:s1, 0:VA])

        def pvb(r0, r1):
            return _dot_nt(wvT[r0:r1, VA:D], xn_s[0, :, VA:D])

        cp_x0a.wait()
        xn_s[0, 0:HX, :] = _layernorm(x_v[0:HX, :].astype(f32)).astype(bf16)
        cp_va.wait()
        wvT[:, 0:VA] = wqkv_v[0:VA, 2 * D:3 * D].T
        paa = pva(0, A0, 0, HX)
        cp_x0b.wait()
        paa = jnp.concatenate([paa, pva(A0, D, 0, HX)], axis=0)
        xn_s[0, HX:TS, :] = _layernorm(x_v[HX:TS, :].astype(f32)).astype(bf16)
        pab = pva(0, A1, HX, TS)
        cp_vb.wait()
        pab = jnp.concatenate([pab, pva(A1, D, HX, TS)], axis=0)
        pa = jnp.concatenate([paa, pab], axis=1)
        wvT[:, VA:D] = wqkv_v[VA:D, 2 * D:3 * D].T
        v0 = pa[0:B1] + pvb(0, B1)
        cp_k.wait()
        wkT[...] = fold(D)
        put_feat(n - 1, PK(0))
        put_lhs(0, jnp.concatenate([v0, pa[B1:D] + pvb(B1, D)], axis=0))
        cp_q.wait()
        cp_x(1).wait()
        wqT[...] = fold(0)
        PQ(0)
        put_kv([_dot_nt(lhs_s[0, KV_OFF[i]:KV_OFF[i + 1], :], fq_s[n - 1, 128 * i:128 * i + 128, :])
                for i in range(NFT)])
        LNPV(1)

        def p1(t, carry):
            cp_x(t + 1).wait()
            fk = PK(t)
            PQ(t)
            PVB(t)
            kv = KV(t, fk)
            LNPV(t + 1)
            put_kv(kv)
            return carry
        lax.fori_loop(1, n - 1, p1, 0)

        fk = PK(n - 1)
        PQ(n - 1)
        PVB(n - 1)
        kv = KV(n - 1, fk)
        cc = _iota((1, 128), 1)
        plus_c = jnp.logical_or(cc % 40 < 16, jnp.logical_and(cc % 40 >= 32, cc % 2 == 0))
        eps_c = jnp.where(plus_c, DEN_EPS, 0.0)
        for i, (r0, r1) in enumerate(KV_W):
            j_c = jnp.where(cc < min(120, 2 * D - 120 * i), cc // 40, -64)
            rr = _iota((KV_L[i], 1), 0)
            dlt = rr - (DH * j_c + (60 * i - r0))
            zrow = rr - KV_J[i] == j_c
            keep = jnp.logical_or(jnp.logical_and(dlt >= 0, dlt < DH), zrow)
            kvT[KV_OFF[i]:KV_OFF[i + 1], :] = (jnp.where(keep, kv[i], 0.0)
                                               + jnp.where(zrow, eps_c, 0.0)).astype(bf16)
        for c in cp_ffn:
            c.wait()

    @pl.when(pl.program_id(0) == 1)
    def _phase2():
        def out_copy(t, c):
            r0, r1, c0, c1 = OCH[c]
            row = pl.multiple_of(t * TS + r0, 64)
            return pltpu.make_async_copy(out_v.at[pl.ds(row, r1 - r0), pl.ds(c0, c1 - c0)],
                                         o_hbm.at[0, pl.ds(row, r1 - r0), pl.ds(c0, c1 - c0)],
                                         osems.at[t * NOC + c])

        def attn_o(t, c0, c1):
            m = c1 - c0
            parts = [_dot(kvT[KV_OFF[i]:KV_OFF[i + 1], :], fq_s[t, 128 * i:128 * i + 128, c0:c1])
                     for i in range(NFT)]
            sub = _iota((8, m), 0)
            lo = sub < 4
            segs, rds = [], []
            for i in range(0, NFT - 1, 2):
                pe, po = parts[i], parts[i + 1]
                segs += [pe[:56], jnp.where(lo, pe[56:64], po[0:8]), po[8:]]
                rd = 1.0 / jnp.where(sub % 4 == 3, 1.0, jnp.where(lo, po[0:8], pe[56:64]))
                rds += [rd[j:j + 1] for j in (4, 5, 6, 0, 1, 2)]
            segs.append(parts[NFT - 1][:40])
            rd = 1.0 / jnp.where(sub < 2, parts[NFT - 1][40:48], 1.0)
            rds += [rd[0:1], rd[1:2]]
            scale = []
            for g in range(NG):
                a0 = jnp.broadcast_to(rds[2 * g], (8, m))
                a1 = jnp.broadcast_to(rds[2 * g + 1], (8, m))
                scale += [a0, a0, jnp.where(lo, a0, a1), a1, a1]
            return (jnp.concatenate(segs, axis=0) * jnp.concatenate(scale, axis=0)).T

        def p2(t, carry):
            row = pl.multiple_of(t * TS, TS)
            ma = TS // NA
            o = jnp.concatenate([attn_o(t, j * ma, (j + 1) * ma) for j in range(NA)], axis=0)
            hs = [x_v[pl.ds(row + r0, WR), :].astype(f32) + _dot(o[r0:r0 + WR].astype(bf16), wo_v[...])
                  for r0 in range(0, TS, WR)]
            hn = jnp.concatenate([_layernorm(h) for h in hs], axis=0)
            h = jnp.concatenate(hs, axis=0)

            def rows(w, par, k, cols):
                return jnp.concatenate([w[r:r + 128, cols] for r in range(128 * par, k, 256)], axis=0)

            def strassen(la, w, k, c):
                a, b = slice(c, c + 128), slice(c + 128, c + 256)
                return _strassen(la, rows(w, 0, k, a), rows(w, 0, k, b), rows(w, 1, k, a), rows(w, 1, k, b))

            he = jnp.concatenate([hn[:, 0:128], hn[:, 256:384]], axis=1)
            ho = jnp.concatenate([hn[:, 128:256], hn[:, 384:512]], axis=1)
            lh = _strassen_lhs(he[:HX], ho[:HX], he[HX:], ho[HX:])
            hr = hn[:, 512:D].astype(bf16)

            def proj(w, c):
                left, right = strassen(lh, w, 512, c)
                return left + _dot(hr, w[512:D, c:c + 128]), right + _dot(hr, w[512:D, c + 128:c + 256])

            al, ar = [], []
            for c in range(0, F, 256):
                (gl, gr), (ul, ur) = proj(wg_v, c), proj(wu_v, c)
                al.append(_gelu(gl) * ul)
                ar.append(_gelu(gr) * ur)
            act = jnp.concatenate([x for pair in zip(al, ar) for x in pair], axis=1)

            ae, ao = jnp.concatenate(al, axis=1), jnp.concatenate(ar, axis=1)
            la = _strassen_lhs(ae[:HX], ao[:HX], ae[HX:], ao[HX:])
            for k, c in enumerate((0, 256)):
                left, right = strassen(la, wd_v, F, c)
                out_v[pl.ds(row, TS), c:c + 256] = (
                    h[:, c:c + 256] + jnp.concatenate([left, right], axis=1)).astype(bf16)
                out_copy(t, k).start()
            for k, (r0, r1, _, _) in enumerate(OCH[2:]):
                y = _dot(act[r0:r1].astype(bf16), wd_v[:, 512:D])
                out_v[pl.ds(pl.multiple_of(row + r0, 64), r1 - r0), 512:D] = (h[r0:r1, 512:D] + y).astype(bf16)
                out_copy(t, 2 + k).start()
            return carry

        lax.fori_loop(0, n, p2, 0)
        for t in range(n):
            for c in range(NOC):
                out_copy(t, c).wait()


_SCRATCH = [
    pltpu.VMEM((S, D), bf16),
    pltpu.VMEM((D, 3 * D), bf16),
    pltpu.VMEM((DH, DH, H), bf16),
    pltpu.VMEM((D, D), bf16),
    pltpu.VMEM((D, F), bf16),
    pltpu.VMEM((D, F), bf16),
    pltpu.VMEM((F, D), bf16),
    pltpu.VMEM((S, D), bf16),
    pltpu.VMEM((NL, D), bf16),
    pltpu.VMEM((D, D), bf16),
    pltpu.VMEM((NL, D), bf16),
    pltpu.VMEM((D, D), bf16),
    pltpu.VMEM((2, TS, D), bf16),
    pltpu.VMEM((KV_OFF[-1], 128), bf16),
    pltpu.VMEM((KV_OFF[-1], 128), f32),
    pltpu.VMEM((FOLD_OFF[-1], 128), bf16),
    pltpu.VMEM((2, KV_OFF[-1], TS), bf16),
    pltpu.VMEM((NTILE, NFT * 128, TS), bf16),
    pltpu.SemaphoreType.DMA((10 + NTILE,)),
    pltpu.SemaphoreType.DMA((NTILE * NOC,)),
]


def _compiler_params():
    kw = dict(dimension_semantics=("arbitrary",), vmem_limit_bytes=100 * 1024 * 1024,
              disable_bounds_checks=True, disable_semaphore_checks=True)
    known = {f.name for f in dataclasses.fields(pltpu.CompilerParams)}
    return pltpu.CompilerParams(**{k: v for k, v in kw.items() if k in known})


@jax.jit
def pallas_sequential_preLN__linear_kernel_hedgehog__geglu_ffn__prompt_kernel(
    A_x: jax.Array,
    A_wqkv: jax.Array,
    A_w_phi: jax.Array,
    A_wo: jax.Array,
    B_x: jax.Array,
    B_w_gate: jax.Array,
    B_w_up: jax.Array,
    B_w_down: jax.Array,
):
    del B_x
    return pl.pallas_call(
        _kernel,
        out_shape=jax.ShapeDtypeStruct(A_x.shape, A_x.dtype),
        grid=(2,),
        in_specs=[pl.BlockSpec(memory_space=pl.ANY)] * 7,
        out_specs=pl.BlockSpec(memory_space=pl.ANY),
        scratch_shapes=_SCRATCH,
        compiler_params=_compiler_params(),
    )(A_x, A_wqkv, jnp.transpose(A_w_phi, (1, 2, 0)), A_wo, B_w_gate, B_w_up, B_w_down)
```
